```python
import os as _os
_os.environ.setdefault("JAX_PLATFORMS", "cpu")
import jax
import jax.numpy as jnp

def _softmax(x, axis=-1):
    return jax.nn.softmax(x, axis=axis)
def _gelu(x):
    return jax.nn.gelu(x, approximate=True)
def _silu(x):
    return jax.nn.silu(x)
def _sigmoid(x):
    return jax.nn.sigmoid(x)
def _layernorm(x, axis=-1, eps=1e-5):
    m = jnp.mean(x, axis=axis, keepdims=True)
    v = jnp.var(x, axis=axis, keepdims=True)
    return (x - m) / jnp.sqrt(v + eps)
def _scatter_add(tgt, idx, src, axis=0):
    return tgt.at[idx].add(src)
def _segment_sum(src, seg, n):
    return jax.ops.segment_sum(src, seg, n)
class _Rng:
    def __init__(self, key):
        self._k = key
    def _next(self):
        self._k, sub = jax.random.split(self._k)
        return sub
    def normal(self, shape):
        return jax.random.normal(self._next(), shape, dtype=jnp.bfloat16)
    def randint(self, lo, hi, shape):
        return jax.random.randint(self._next(), shape, lo, hi, dtype=jnp.int32)
    def uniform(self, shape, lo=0.0, hi=1.0):
        return jax.random.uniform(self._next(), shape, jnp.bfloat16, lo, hi)
    def permutation(self, n):
        return jax.random.permutation(self._next(), n)


kernel_name = 'gated_mix__grouped_kv_mqa__swiglu_ffn__prompt'

def setup_inputs():
    _rng = _Rng(jax.random.key(int.from_bytes(__import__("os").urandom(4), "little")))
    _w = (lambda a: (lambda t: t.astype(jnp.bfloat16) if jnp.issubdtype(t.dtype, jnp.floating) else t)(jnp.asarray(a)))
    def _A_setup():
        B, S, D, H = 1, 2048, 512, 32
        Dh = D // H
        return {
            "x": _w((lambda *s: _rng.normal(s) * 0.05)(B, S, D)),
            "wq": _w((lambda *s: _rng.normal(s) * 0.4)(D, H * Dh)),
            "wk": _w((lambda *s: _rng.normal(s) * 0.4)(D, Dh)),
            "wv": _w((lambda *s: _rng.normal(s) * 0.05)(D, Dh)),
            "wo": _w((lambda *s: _rng.normal(s) * 0.05)(H * Dh, D)),
        }
    _A_in = _A_setup()

    def _B_setup():
        B, S, D, F = 1, 2048, 512, 1792
        return {
            "x": _w((lambda *s: _rng.normal(s) * 0.05)(B, S, D)),
            "w_gate": _w((lambda *s: _rng.normal(s) * 0.05)(D, F)),
            "w_up": _w((lambda *s: _rng.normal(s) * 0.05)(D, F)),
            "w_down": _w((lambda *s: _rng.normal(s) * 0.05)(F, D)),
        }
    _B_in = _B_setup()

    return {
        "A_x": _A_in["x"],
        "A_wq": _A_in["wq"],
        "A_wk": _A_in["wk"],
        "A_wv": _A_in["wv"],
        "A_wo": _A_in["wo"],
        "B_x": _B_in["x"],
        "B_w_gate": _B_in["w_gate"],
        "B_w_up": _B_in["w_up"],
        "B_w_down": _B_in["w_down"],
        "gate_w": _w((lambda *s: _rng.normal(s) * 0.05)(512) * 16.0),
    }

def reference(A_x, A_wq, A_wk, A_wv, A_wo, B_x, B_w_gate, B_w_up, B_w_down, gate_w):
    def _A_ref(x, wq, wk, wv, wo):
        B, S, D = x.shape
        H = 32
        Dh = D // H
        q = (lambda x, *d: x.transpose(*d))((x @ wq).reshape(B, S, H, Dh), 0, 2, 1, 3)
        k = x @ wk
        v = x @ wv
        scores = jnp.einsum("bhqd,bkd->bhqk", q, k) * (Dh ** -0.5)
        p = _softmax(scores, axis=-1)
        o = jnp.einsum("bhqk,bkd->bhqd", p, v)
        return (lambda x, *d: x.transpose(*d))(o, 0, 2, 1, 3).reshape(B, S, H * Dh) @ wo

    def _B_ref(x, w_gate, w_up, w_down):
        g = _silu(x @ w_gate)
        u = x @ w_up
        return (g * u) @ w_down

    x = A_x
    g = _sigmoid((x * gate_w).sum(-1, keepdims=True))
    a = _A_ref(x, A_wq, A_wk, A_wv, A_wo)
    b = _B_ref(x, B_w_gate, B_w_up, B_w_down)
    return g * a + (1 - g) * b
```

```python
import math

import jax
import jax.numpy as jnp
import jax.experimental.pallas as pl
import jax.experimental.pallas.tpu as pltpu

S = 2048
D = 512
H = 32
DH = 16
F = 1792

TB = 512
TK = 128
NC = S // TK
G = 4
LAG = 2
KD = 32
FC = 256

QSCALE = (DH ** -0.5) * math.log2(math.e)
SAFE_BOUND = 40.0

_TT = (((0,), (1,)), ((), ()))
_TN = (((0,), (0,)), ((), ()))


def _kernel(x_hbm, wq_hbm, wk_hbm, wv_hbm, wo_hbm, wg_hbm, wu_hbm, wd_hbm,
            gw_ref, o_ref,
            x_v, wq_v, wk_v, wv_v, wo_v, wg_v, wu_v, wd_v,
            kext, vt, kmax2, qext, ot, h_scr, sems):
    step = pl.program_id(0)
    f32, bf16 = jnp.float32, jnp.bfloat16

    srcs = (x_hbm, wk_hbm, wv_hbm, wq_hbm, wo_hbm, wg_hbm, wu_hbm, wd_hbm)
    dsts = (x_v, wk_v, wv_v, wq_v, wo_v, wg_v, wu_v, wd_v)

    def copy(i):
        return pltpu.make_async_copy(srcs[i], dsts[i], sems.at[i])

    @pl.when(step == 0)
    def _prologue():
        for i in range(8):
            copy(i).start()
        for i in range(4):
            copy(i).wait()
        x = x_v[...]
        wk = wk_v[...]
        wkv = jnp.concatenate([wk, wv_v[...]], axis=1)
        kvt = jax.lax.dot_general(wkv, x, _TT, preferred_element_type=f32)
        vt[...] = kvt[DH:, :].astype(bf16)
        kt = kvt[:DH, :].astype(bf16).astype(f32)
        kn2 = jnp.sum(kt * kt, axis=0, keepdims=True)
        kmax2[...] = jnp.broadcast_to(
            jnp.max(kn2, axis=1, keepdims=True), kmax2.shape)
        wk_ext = jnp.concatenate([wk, jnp.zeros_like(wk)], axis=1)
        k = jnp.dot(x, wk_ext, preferred_element_type=f32)
        lane = jax.lax.broadcasted_iota(jnp.int32, k.shape, 1)
        ones = jnp.logical_and(lane >= DH, lane < DH + 3)
        kext[...] = jnp.where(ones, 1.0, k).astype(bf16)

    row0 = pl.multiple_of(step * TB, TB)
    xb = x_v[pl.ds(row0, TB), :]

    qt = jax.lax.dot_general(wq_v[...], xb, _TT, preferred_element_type=f32)
    qs = (qt * QSCALE).astype(bf16).reshape(H, DH, TB)
    qf = qs.astype(f32)
    qn2 = jnp.sum(qf * qf, axis=1, keepdims=True)
    bound = jnp.sqrt(qn2 * kmax2[0:1, :].reshape(1, 1, TB)) * (1.0 + 2.0 ** -6)
    bound = bound.astype(bf16).astype(f32)
    rid = jax.lax.broadcasted_iota(jnp.int32, (H, DH, TB), 1)
    qext[:, 0:DH, :] = qs
    qext[:, DH:KD, :] = jnp.where(rid == 0, -bound, 0.0).astype(bf16)
    unsafe = jnp.logical_not(jnp.max(bound) <= SAFE_BOUND)

    @pl.when(unsafe)
    def _true_max():
        def head(h, carry):
            q = qext[h, 0:DH, :]

            def chunk(c, m):
                kk = kext[pl.ds(pl.multiple_of(c * TK, TK), TK), 0:DH]
                s = jnp.dot(kk, q, preferred_element_type=f32)
                return jnp.maximum(m, jnp.max(s, axis=0, keepdims=True))

            m = jax.lax.fori_loop(0, NC, chunk,
                                  jnp.full((1, TB), -jnp.inf, f32))
            hi = m.astype(bf16).astype(f32)
            mid = (m - hi).astype(bf16).astype(f32)
            lo = (m - hi - mid).astype(bf16).astype(f32)
            r = jax.lax.broadcasted_iota(jnp.int32, (DH, TB), 0)
            ext = jnp.where(r == 0, -hi,
                            jnp.where(r == 1, -mid,
                                      jnp.where(r == 2, -lo, 0.0)))
            qext[h, DH:KD, :] = ext.astype(bf16)
            return carry

        jax.lax.fori_loop(0, H, head, 0)

    def attn_body(it, carry):
        ps, osum, lsum = {}, {}, {}
        T = G * NC
        for t in range(T + LAG):
            if t < T:
                g, c = divmod(t, NC)
                q = qext[it * G + g]
                s = jnp.dot(kext[c * TK:(c + 1) * TK, :], q,
                            preferred_element_type=f32)
                p = jnp.exp2(s)
                r = p.reshape(TK // 8, 8, TB).sum(axis=0)
                lsum[g] = r + lsum[g] if c else r
                ps[t] = p.astype(bf16)
            d = t - LAG
            if d >= 0:
                g, c = divmod(d, NC)
                pv = jnp.dot(vt[:, c * TK:(c + 1) * TK], ps.pop(d),
                             preferred_element_type=f32)
                osum[g] = pv + osum[g] if c else pv
                if c == NC - 1:
                    l = lsum.pop(g).sum(axis=0, keepdims=True)
                    o = osum.pop(g) / l
                    hrow = pl.multiple_of((it * G + g) * DH, DH)
                    ot[pl.ds(hrow, DH), :] = o.astype(bf16)
        return carry

    jax.lax.fori_loop(0, H // G, attn_body, 0)

    @pl.when(step == 0)
    def _wait_weights():
        for i in range(4, 8):
            copy(i).wait()

    for c in range(F // FC):
        gcol = jnp.dot(xb, wg_v[:, c * FC:(c + 1) * FC],
                       preferred_element_type=f32)
        ucol = jnp.dot(xb, wu_v[:, c * FC:(c + 1) * FC],
                       preferred_element_type=f32)
        h_scr[:, c * FC:(c + 1) * FC] = (
            gcol * jax.nn.sigmoid(gcol) * ucol).astype(bf16)
    a = jax.lax.dot_general(ot[...], wo_v[...], _TN,
                            preferred_element_type=f32)
    b = jnp.dot(h_scr[...], wd_v[...], preferred_element_type=f32)
    gate = jax.nn.sigmoid(jnp.sum(
        xb.astype(f32) * gw_ref[...].astype(f32), axis=1, keepdims=True))
    o_ref[...] = (gate * a + (1.0 - gate) * b).astype(o_ref.dtype)


@jax.jit
def pallas_gated_mix__grouped_kv_mqa__swiglu_ffn__prompt_kernel(
    A_x: jax.Array,
    A_wq: jax.Array,
    A_wk: jax.Array,
    A_wv: jax.Array,
    A_wo: jax.Array,
    B_x: jax.Array,
    B_w_gate: jax.Array,
    B_w_up: jax.Array,
    B_w_down: jax.Array,
    gate_w: jax.Array,
):
    del B_x
    bf16 = jnp.bfloat16
    any_spec = pl.BlockSpec(memory_space=pl.ANY)
    out = pl.pallas_call(
        _kernel,
        grid=(S // TB,),
        in_specs=[any_spec] * 8 + [pl.BlockSpec((1, D), lambda i: (0, 0))],
        out_specs=pl.BlockSpec((TB, D), lambda i: (i, 0)),
        out_shape=jax.ShapeDtypeStruct((S, D), A_x.dtype),
        scratch_shapes=[
            pltpu.VMEM((S, D), bf16),
            pltpu.VMEM((D, D), bf16),
            pltpu.VMEM((D, DH), bf16),
            pltpu.VMEM((D, DH), bf16),
            pltpu.VMEM((D, D), bf16),
            pltpu.VMEM((D, F), bf16),
            pltpu.VMEM((D, F), bf16),
            pltpu.VMEM((F, D), bf16),
            pltpu.VMEM((S, KD), bf16),
            pltpu.VMEM((DH, S), bf16),
            pltpu.VMEM((8, TB), jnp.float32),
            pltpu.VMEM((H, KD, TB), bf16),
            pltpu.VMEM((D, TB), bf16),
            pltpu.VMEM((TB, F), bf16),
            pltpu.SemaphoreType.DMA((8,)),
        ],
        compiler_params=pltpu.CompilerParams(
            dimension_semantics=("arbitrary",),
            vmem_limit_bytes=100 * 1024 * 1024,
        ),
    )(A_x.reshape(S, D), A_wq, A_wk, A_wv, A_wo,
      B_w_gate, B_w_up, B_w_down, gate_w.reshape(1, D))
    return out.reshape(A_x.shape)
```

```python
import math

import jax
import jax.numpy as jnp
import jax.experimental.pallas as pl
import jax.experimental.pallas.tpu as pltpu

S = 2048
D = 512
H = 32
DH = 16
F = 1792

TB = 512
NB = S // TB
NL = TB // 128
TK = 128
NC = S // TK
G = 8
LAG = 2
KD = 32
FC = 256
R = 16
POS = (4, 7, 10, 13)

QSCALE = (DH ** -0.5) * math.log2(math.e)
SAFE_BOUND = 40.0

_NT = (((1,), (1,)), ((), ()))
_TN = (((0,), (0,)), ((), ()))


def _kernel(x_hbm, wq_hbm, wkt_hbm, wvt_hbm, wo_hbm, wg_hbm, wu_hbm, wd_hbm,
            gw_ref, o_ref,
            x_v, wq_v, wkt_v, wvt_v, wo_v, wg_v, wu_v, wd_v,
            kext, vt, kb, qext, qf32, negm, ot, h_scr,
            p_car, o_car, l_car, sems):
    step = pl.program_id(0)
    f32, bf16 = jnp.float32, jnp.bfloat16

    srcs = (wkt_hbm, wvt_hbm, wq_hbm, wo_hbm, wg_hbm, wu_hbm, wd_hbm)
    dsts = (wkt_v, wvt_v, wq_v, wo_v, wg_v, wu_v, wd_v)

    def copy(i):
        return pltpu.make_async_copy(srcs[i], dsts[i], sems.at[i])

    def xcopy(b):
        return pltpu.make_async_copy(x_hbm.at[pl.ds(b * TB, TB), :],
                                     x_v.at[pl.ds(b * TB, TB), :],
                                     sems.at[7 + b])

    @pl.when(step == 0)
    def _prologue():
        for i in range(3):
            copy(i).start()
        for b in range(NB):
            xcopy(b).start()
        p_car[...] = jnp.zeros_like(p_car)
        o_car[...] = jnp.zeros_like(o_car)
        l_car[...] = jnp.ones_like(l_car)
        er = jax.lax.broadcasted_iota(jnp.int32, (KD, DH * 128), 0)
        ec = jax.lax.broadcasted_iota(jnp.int32, (KD, DH * 128), 1)
        e = jnp.where(er == (ec >> 7), 1.0, 0.0).astype(bf16)
        hr = jax.lax.broadcasted_iota(jnp.int32, (H, D), 0)
        hc = jax.lax.broadcasted_iota(jnp.int32, (H, D), 1)
        sel = jnp.where(hr == (hc >> 4), 1.0, 0.0).astype(bf16)
        for i in range(3):
            copy(i).wait()
        wqt = wq_v[...].T
        wkvt = jnp.concatenate([wkt_v[...], wvt_v[...]], axis=0)
        cpb = TB // TK

        def kv_block(b):
            xb = x_v[b * TB:(b + 1) * TB, :]
            kvt = jax.lax.dot_general(wkvt, xb, _NT,
                                      preferred_element_type=f32)
            vt[:, b * TB:(b + 1) * TB] = pltpu.bitcast(
                kvt[DH:, :].astype(bf16), jnp.uint32)
            kt = kvt[:DH, :].astype(bf16).astype(f32)
            ktx = jnp.concatenate(
                [kt, jnp.ones((8, TB), f32), jnp.zeros((8, TB), f32)], axis=0)
            kx = ktx.T.astype(bf16)
            kext[b * TB // 2:(b + 1) * TB // 2, :] = pltpu.bitcast(
                kx, jnp.uint32)
            kv = jnp.concatenate(
                [kx[(c + 1) * TK - R:(c + 1) * TK, :] for c in range(cpb)],
                axis=0)
            return kv, jnp.sum(kt * kt, axis=0, keepdims=True)

        def kb_block(b, kv):
            kb[b * cpb * R:(b + 1) * cpb * R, :] = jnp.dot(
                kv, e, preferred_element_type=f32)

        def q_block(b):
            xb = x_v[b * TB:(b + 1) * TB, :]
            qt = jax.lax.dot_general(wqt, xb, _NT, preferred_element_type=f32)
            qs = (qt * QSCALE).astype(bf16)
            qf = qs.astype(f32)
            qext[b, :, 0:DH, :] = qs.reshape(H, DH, TB)
            qf32[b] = qf.reshape(H, DH, TB)
            return (qf * qf).astype(bf16)

        gi = jax.lax.broadcasted_iota(jnp.int32, (H // 8, 8, 8, TB), 1)
        ri = jax.lax.broadcasted_iota(jnp.int32, (H // 8, 8, 8, TB), 2)

        def shift_block(b, q2, kmax2):
            qn2 = jnp.dot(sel, q2, preferred_element_type=f32)
            bound = jnp.sqrt(qn2 * kmax2)
            bound = (bound * (1.0 + 2.0 ** -6)).astype(bf16).astype(f32)
            nb = (-bound).reshape(H // 8, 8, TB)
            negm[b] = nb
            ext = jnp.where(gi == ri, nb[:, None, :, :], 0.0).reshape(H, 8, TB)
            qext[b, :, DH:KD, :] = jnp.concatenate(
                [ext, jnp.zeros_like(ext)], axis=1).astype(bf16)
            return bound

        xcopy(0).wait()
        kvs = [kv_block(0)]
        q2 = q_block(0)
        for b in range(1, NB):
            xcopy(b).wait()
        for i in range(3, 7):
            copy(i).start()
        kvs += [kv_block(b) for b in range(1, NB)]
        km = kvs[0][1]
        for b in range(1, NB):
            km = jnp.maximum(km, kvs[b][1])
        kmax2 = jnp.max(km, axis=1, keepdims=True)
        bmax = None
        for b in range(NB):
            q2_next = q_block(b + 1) if b + 1 < NB else None
            bound = shift_block(b, q2, kmax2)
            if b + 2 == NB:
                for bb in range(NB):
                    kb_block(bb, kvs[bb][0])
            bmax = bound if bmax is None else jnp.maximum(bmax, bound)
            q2 = q2_next
        unsafe = jnp.logical_not(jnp.max(bmax) <= SAFE_BOUND)

        @pl.when(unsafe)
        def _true_max():
            def group(n, carry):
                b, hg = n // (H // 8), n % (H // 8)
                for g in range(8):
                    q = qext[b, hg * 8 + g, 0:DH, :]

                    def chunk(c, m):
                        kk = pltpu.bitcast(kext[pl.ds(pl.multiple_of(c * TK // 2, TK // 2), TK // 2), :], bf16)[:, 0:DH]
                        s = jnp.dot(kk, q, preferred_element_type=f32)
                        return jnp.maximum(
                            m, jnp.max(s, axis=0, keepdims=True))

                    m = jax.lax.fori_loop(0, NC, chunk,
                                          jnp.full((1, TB), -jnp.inf, f32))
                    hi = m.astype(bf16).astype(f32)
                    mid = (m - hi).astype(bf16).astype(f32)
                    lo = (m - hi - mid).astype(bf16).astype(f32)
                    r = jax.lax.broadcasted_iota(jnp.int32, (DH, TB), 0)
                    ex = jnp.where(r == 0, -hi,
                                   jnp.where(r == 1, -mid,
                                             jnp.where(r == 2, -lo, 0.0)))
                    qext[b, hg * 8 + g, DH:KD, :] = ex.astype(bf16)
                    negm[b, hg, g:g + 1, :] = -(hi + mid + lo)
                return carry

            jax.lax.fori_loop(0, NB * (H // 8), group, 0)

    def pv_dot(c, p):
        return jnp.dot(pltpu.bitcast(vt[:, c * TK:(c + 1) * TK], bf16), p,
                       preferred_element_type=f32)

    def finish(o, l, hrow):
        o = o / l.sum(axis=0, keepdims=True)
        ot[pl.ds(hrow, DH), :] = o.astype(bf16)

    def attn_body(it, carry):
        ps, lsum = {}, {}
        osum = {-1: o_car[...]}
        T = G * NC

        def vpu_rows(g, c, j):
            h = it * G + g
            lanes = slice(j * 128, (j + 1) * 128)
            shift = negm[step, it * (G // 8) + g // 8, g % 8:g % 8 + 1, lanes]
            accs = [jnp.broadcast_to(shift, (8, 128))] * (R // 8)
            for d in range(DH):
                qrow = jnp.broadcast_to(qf32[step, h, d:d + 1, lanes], (8, 128))
                for r in range(R // 8):
                    r0 = c * R + r * 8
                    accs[r] = accs[r] + (
                        kb[r0:r0 + 8, d * 128:(d + 1) * 128] * qrow)
            return [jnp.exp2(a) for a in accs]

        for t in range(T):
            g, c = divmod(t, NC)
            s = jnp.dot(pltpu.bitcast(kext[c * TK // 2:((c + 1) * TK - R) // 2, :], bf16),
                        qext[step, it * G + g], preferred_element_type=f32)
            pm = jnp.exp2(s)
            vcols = []
            for j in range(NL):
                pv_rows = vpu_rows(g, c, j)
                acc = lsum.get((g, j))
                for n in range((TK - R) // 8):
                    if n == POS[j]:
                        for w in pv_rows:
                            acc = acc + w
                    v = pm[n * 8:(n + 1) * 8, j * 128:(j + 1) * 128]
                    acc = v if acc is None else acc + v
                lsum[(g, j)] = acc
                vcols.append(jnp.concatenate(pv_rows, axis=0))
            p = jnp.concatenate([pm, jnp.concatenate(vcols, axis=1)], axis=0)
            ps[t] = p.astype(bf16)

            g, c = divmod(t - LAG, NC)
            pv = pv_dot(c, ps.pop(t - LAG) if t >= LAG else p_car[t])
            osum[g] = pv + osum[g] if c else pv
            if c == NC - 1:
                if g >= 0:
                    l = jnp.concatenate(
                        [lsum.pop((g, j)) for j in range(NL)], axis=1)
                    hrow = (it * G + g) * DH
                else:
                    l = l_car[...]
                    hrow = jnp.where(it == 0, H * DH, (it * G - 1) * DH)
                finish(osum.pop(g), l, pl.multiple_of(hrow, DH))
        for n in range(LAG):
            p_car[n] = ps.pop(T - LAG + n)
        o_car[...] = osum.pop(G - 1)
        l_car[...] = jnp.concatenate(
            [lsum.pop((G - 1, j)) for j in range(NL)], axis=1)
        return carry

    jax.lax.fori_loop(0, H // G, attn_body, 0)

    @pl.when(step == 0)
    def _wait_weights():
        for i in range(3, 7):
            copy(i).wait()

    xb = x_v[pl.ds(pl.multiple_of(step * TB, TB), TB), :]
    for c in range(F // FC):
        gcol = jnp.dot(xb, wg_v[:, c * FC:(c + 1) * FC],
                       preferred_element_type=f32)
        if c == 0:
            o = o_car[...]
            for n in range(LAG):
                o = o + pv_dot(NC - LAG + n, p_car[n])
            finish(o, l_car[...], (H - 1) * DH)
        ucol = jnp.dot(xb, wu_v[:, c * FC:(c + 1) * FC],
                       preferred_element_type=f32)
        hg = 0.5 * gcol
        h_scr[:, c * FC:(c + 1) * FC] = (
            (hg * jnp.tanh(hg) + hg) * ucol).astype(bf16)
    a = jax.lax.dot_general(ot[0:D, :], wo_v[...], _TN,
                            preferred_element_type=f32)
    b = jnp.dot(h_scr[...], wd_v[...], preferred_element_type=f32)
    gw = gw_ref[...].astype(f32).reshape(1, D)
    gate = jax.nn.sigmoid(jnp.sum(xb.astype(f32) * gw, axis=1, keepdims=True))
    o_ref[...] = (gate * a + (1.0 - gate) * b).astype(o_ref.dtype)


@jax.jit
def pallas_gated_mix__grouped_kv_mqa__swiglu_ffn__prompt_kernel(
    A_x: jax.Array,
    A_wq: jax.Array,
    A_wk: jax.Array,
    A_wv: jax.Array,
    A_wo: jax.Array,
    B_x: jax.Array,
    B_w_gate: jax.Array,
    B_w_up: jax.Array,
    B_w_down: jax.Array,
    gate_w: jax.Array,
):
    del B_x
    bf16, f32 = jnp.bfloat16, jnp.float32
    any_spec = pl.BlockSpec(memory_space=pl.ANY)
    out = pl.pallas_call(
        _kernel,
        grid=(NB,),
        in_specs=[any_spec] * 8 + [pl.BlockSpec((D,), lambda i: (0,))],
        out_specs=pl.BlockSpec((TB, D), lambda i: (i, 0)),
        out_shape=jax.ShapeDtypeStruct((S, D), A_x.dtype),
        scratch_shapes=[
            pltpu.VMEM((S, D), bf16),
            pltpu.VMEM((D, D), bf16),
            pltpu.VMEM((DH, D), bf16),
            pltpu.VMEM((DH, D), bf16),
            pltpu.VMEM((D, D), bf16),
            pltpu.VMEM((D, F), bf16),
            pltpu.VMEM((D, F), bf16),
            pltpu.VMEM((F, D), bf16),
            pltpu.VMEM((S // 2, KD), jnp.uint32),
            pltpu.VMEM((DH // 2, S), jnp.uint32),
            pltpu.VMEM((NC * R, DH * 128), f32),
            pltpu.VMEM((NB, H, KD, TB), bf16),
            pltpu.VMEM((NB, H, DH, TB), f32),
            pltpu.VMEM((NB, H // 8, 8, TB), f32),
            pltpu.VMEM((D + DH, TB), bf16),
            pltpu.VMEM((TB, F), bf16),
            pltpu.VMEM((LAG, TK, TB), bf16),
            pltpu.VMEM((DH, TB), f32),
            pltpu.VMEM((8, TB), f32),
            pltpu.SemaphoreType.DMA((7 + NB,)),
        ],
        compiler_params=pltpu.CompilerParams(
            dimension_semantics=("arbitrary",),
            vmem_limit_bytes=100 * 1024 * 1024,
        ),
    )(A_x.reshape(S, D), A_wq, A_wk.T, A_wv.T, A_wo,
      B_w_gate, B_w_up, B_w_down, gate_w)
    return out.reshape(A_x.shape)
```

```python
import math

import jax
import jax.numpy as jnp
import jax.experimental.pallas as pl
import jax.experimental.pallas.tpu as pltpu

S = 2048
D = 512
H = 32
DH = 16
F = 1792

TB = 512
NB = S // TB
NL = TB // 128
TK = 128
NC = S // TK
G = 8
LAG = 2
KD = 32
FC = 256
NF = F // FC
NO = 4
RO = TB // NO

R = 16
BIG = (2, 5, 8, 11, 14)
NBIG = len(BIG)
POS = (4, 7, 10, 13)
POSB = (1, 5, 8, 11)
WTS = (120, 80, 110, 100)
NQS = (32, 48, 16)
H0 = 12
HS = 8

QSCALE = (DH ** -0.5) * math.log2(math.e)
SAFE_BOUND = 40.0

_NT = (((1,), (1,)), ((), ()))
_TN = (((0,), (0,)), ((), ()))


def _kernel(x_hbm, wq_hbm, wkt_hbm, wvt_hbm, wo_hbm, wg_hbm, wu_hbm, wd_hbm,
            gw_ref, o_hbm,
            x_v, wq_v, wkt_v, wvt_v, wo_v, wg_v, wu_v, wd_v,
            kext, vt, kb, qext, qf32, negm, ot,
            p_car, o_car, l_car, s_pre, obuf, sems):
    step = pl.program_id(0)
    f32, bf16, u32 = jnp.float32, jnp.bfloat16, jnp.uint32

    srcs = (wkt_hbm, wvt_hbm, wq_hbm, wo_hbm, wg_hbm, wu_hbm, wd_hbm)
    dsts = (wkt_v, wvt_v, wq_v, wo_v, wg_v, wu_v, wd_v)

    def copy(i):
        return pltpu.make_async_copy(srcs[i], dsts[i], sems.at[i])

    def xcopy(b):
        return pltpu.make_async_copy(x_hbm.at[pl.ds(b * TB, TB), :],
                                     x_v.at[pl.ds(b * TB, TB), :],
                                     sems.at[7 + b])

    def ocopy(blk, r):
        return pltpu.make_async_copy(
            obuf.at[pl.ds(r * RO, RO), :],
            o_hbm.at[pl.ds(pl.multiple_of(blk * TB + r * RO, RO), RO), :],
            sems.at[7 + NB + r])

    never = jax.lax.broadcasted_iota(jnp.int32, (8, 128), 0) < -step

    def vpu_scores(blk, h, k0, j, init=None, anchor=None):
        acc = init
        for d in range(DH):
            qrow = qf32[blk, h, d:d + 1, j * 128:(j + 1) * 128]
            if d == 0 and anchor is not None:
                qrow = jnp.where(never, anchor,
                                 jnp.broadcast_to(qrow, (8, 128)))
                qrow = jnp.concatenate([qrow, qrow], axis=0)
            pr = kb[k0:k0 + R, d * 128:(d + 1) * 128] * qrow
            acc = pr if acc is None else acc + pr
        return acc

    def release(blk, jobs, res):
        nr, ncol = res.shape[0] // 8, res.shape[1] // 128
        for m, (h, i, half, j) in enumerate(jobs):
            r, jn = (m * nr) // len(jobs), m % ncol
            k0 = (NC + i) * R if half == 0 else BIG[i] * R
            s_pre[h, i, half * R:(half + 1) * R, j * 128:(j + 1) * 128] = (
                vpu_scores(blk, h, k0, j, anchor=res[
                    r * 8:(r + 1) * 8, jn * 128:(jn + 1) * 128]))

    @pl.when(step == 0)
    def _prologue():
        for i in range(3):
            copy(i).start()
        xcopy(0).start()
        p_car[...] = jnp.zeros_like(p_car)
        o_car[...] = jnp.zeros_like(o_car)
        l_car[...] = jnp.ones_like(l_car)
        hr = jax.lax.broadcasted_iota(jnp.int32, (H, D), 0)
        hc = jax.lax.broadcasted_iota(jnp.int32, (H, D), 1)
        sel = jnp.where(hr == (hc >> 4), 1.0, 0.0).astype(bf16)
        for i in range(3):
            copy(i).wait()
        for b in range(1, NB):
            xcopy(b).start()
        wqt = wq_v[...].T
        wkvt = jnp.concatenate([wkt_v[...], wvt_v[...]], axis=0)
        cpb = TB // TK
        kxe = []

        def kv_block(b):
            xb = x_v[b * TB:(b + 1) * TB, :]
            kvt = jax.lax.dot_general(wkvt, xb, _NT,
                                      preferred_element_type=f32)
            vt[:, b * TB:(b + 1) * TB] = pltpu.bitcast(
                kvt[DH:, :].astype(bf16), u32)
            kt = kvt[:DH, :].astype(bf16).astype(f32)
            ktx = jnp.concatenate(
                [kt, jnp.ones((8, TB), f32), jnp.zeros((8, TB), f32)], axis=0)
            kxf = ktx.T
            kx = kxf.astype(bf16)
            kext[b * TB // 2:(b + 1) * TB // 2, :] = pltpu.bitcast(kx, u32)
            for c in range(cpb):
                cg = b * cpb + c
                vpu_rows = [(cg, (c + 1) * TK - R)]
                if cg in BIG:
                    kxe.append(kx[(c + 1) * TK - 2 * R:(c + 1) * TK - R, :])
                    vpu_rows.append((NC + BIG.index(cg), (c + 1) * TK - 2 * R))
                for slot, r0 in vpu_rows:
                    for d in range(DH):
                        kb[slot * R:(slot + 1) * R, d * 128:(d + 1) * 128] = (
                            jnp.broadcast_to(kxf[r0:r0 + R, d:d + 1], (R, 128)))
            return jnp.sum(kt * kt, axis=0, keepdims=True)

        jobs0 = [(h, i, 1, 0) for i in range(NBIG) for h in range(H)]

        def q_block(b):
            xb = x_v[b * TB:(b + 1) * TB, :]
            qt = jax.lax.dot_general(wqt, xb, _NT, preferred_element_type=f32)
            if b:
                release(0, jobs0[sum(NQS[:b - 1]):sum(NQS[:b])], qt)
            qs = (qt * QSCALE).astype(bf16)
            qf = qs.astype(f32)
            qext[b, :, 0:DH, :] = qs.reshape(H, DH, TB)
            qf32[b] = qf.reshape(H, DH, TB)
            return (qf * qf).astype(bf16)

        gi = jax.lax.broadcasted_iota(jnp.int32, (H // 8, 8, 8, TB), 1)
        ri = jax.lax.broadcasted_iota(jnp.int32, (H // 8, 8, 8, TB), 2)

        def shift_block(b, q2, kmax2):
            qn2 = jnp.dot(sel, q2, preferred_element_type=f32)
            bound = jnp.sqrt(qn2 * kmax2)
            bound = (bound * (1.0 + 2.0 ** -6)).astype(bf16).astype(f32)
            nb = (-bound).reshape(H // 8, 8, TB)
            negm[b] = nb
            ext = jnp.where(gi == ri, nb[:, None, :, :], 0.0).reshape(H, 8, TB)
            qext[b, :, DH:KD, :] = jnp.concatenate(
                [ext, jnp.zeros_like(ext)], axis=1).astype(bf16)
            return bound

        xcopy(0).wait()
        km = kv_block(0)
        q2 = q_block(0)
        for b in range(1, NB):
            xcopy(b).wait()
        for i in range(3, 7):
            copy(i).start()
        for b in range(1, NB):
            km = jnp.maximum(km, kv_block(b))
        kmax2 = jnp.max(km, axis=1, keepdims=True)
        bmax = None
        for b in range(NB - 1):
            q2_next = q_block(b + 1)
            bound = shift_block(b, q2, kmax2)
            bmax = bound if bmax is None else jnp.maximum(bmax, bound)
            q2 = q2_next
        ke = jnp.concatenate(kxe, axis=0)[:, 0:DH]
        rest = jobs0[sum(NQS):]
        for h in range(H):
            se = jnp.dot(ke, qext[0, h, 0:DH, :], preferred_element_type=f32)
            s_pre[h, :, 0:R, :] = se.reshape(NBIG, R, TB)
            if h >= H0:
                release(0, rest[(h - H0) * len(rest) // (H - 2 - H0):
                                (h - H0 + 1) * len(rest) // (H - 2 - H0)], se)
            if h == HS:
                bmax = jnp.maximum(bmax, shift_block(NB - 1, q2, kmax2))
        unsafe = jnp.logical_not(jnp.max(bmax) <= SAFE_BOUND)

        @pl.when(unsafe)
        def _true_max():
            def group(n, carry):
                b, hg = n // (H // 8), n % (H // 8)
                for g in range(8):
                    q = qext[b, hg * 8 + g, 0:DH, :]

                    def chunk(c, m):
                        r0 = pl.multiple_of(c * (TK // 2), TK // 2)
                        kk = pltpu.bitcast(kext[pl.ds(r0, TK // 2), :], bf16)
                        s = jnp.dot(kk[:, 0:DH], q, preferred_element_type=f32)
                        return jnp.maximum(
                            m, jnp.max(s, axis=0, keepdims=True))

                    m = jax.lax.fori_loop(0, NC, chunk,
                                          jnp.full((1, TB), -jnp.inf, f32))
                    hi = m.astype(bf16).astype(f32)
                    mid = (m - hi).astype(bf16).astype(f32)
                    lo = (m - hi - mid).astype(bf16).astype(f32)
                    r = jax.lax.broadcasted_iota(jnp.int32, (DH, TB), 0)
                    ex = jnp.where(r == 0, -hi,
                                   jnp.where(r == 1, -mid,
                                             jnp.where(r == 2, -lo, 0.0)))
                    qext[b, hg * 8 + g, DH:KD, :] = ex.astype(bf16)
                    negm[b, hg, g:g + 1, :] = -(hi + mid + lo)
                return carry

            jax.lax.fori_loop(0, NB * (H // 8), group, 0)

    def pv_dot(c, p):
        return jnp.dot(pltpu.bitcast(vt[:, c * TK:(c + 1) * TK], bf16), p,
                       preferred_element_type=f32)

    def finish(o, l, hrow):
        o = o * (1.0 / l.sum(axis=0, keepdims=True))
        ot[pl.ds(hrow, DH), :] = o.astype(bf16)

    def attn_body(it, carry):
        ps, lsum = {}, {}
        osum = {-1: o_car[...]}
        T = G * NC

        for t in range(T):
            g, c = divmod(t, NC)
            h = it * G + g
            big = c in BIG
            nm = TK - (2 * R if big else R)
            s = jnp.dot(
                pltpu.bitcast(kext[c * TK // 2:(c * TK + nm) // 2, :], bf16),
                qext[step, h], preferred_element_type=f32)
            pm = jnp.exp2(s)
            shift = negm[step, it * (G // 8) + g // 8, g % 8:g % 8 + 1, :]
            own = [vpu_scores(step, h, c * R, j,
                              init=shift[:, j * 128:(j + 1) * 128])
                   for j in range(1 if big else 0, NL)]
            off = []
            if big:
                i = BIG.index(c)
                pe = jnp.exp2(s_pre[h, i, 0:R, :] + shift)
                own.insert(0, s_pre[h, i, R:2 * R, 0:128] + shift[:, 0:128])
                off.append(pe)
            off.append(jnp.exp2(jnp.concatenate(own, axis=1)))
            pos = POSB if big else POS
            acc = lsum.get(g)
            for n in range(nm // 8):
                if big and n == 1:
                    acc = acc + pe[0:8] + pe[8:16]
                if n in pos:
                    j = pos.index(n)
                    w = off[-1][:, j * 128:(j + 1) * 128]
                    parts = [acc[:, j * 128:(j + 1) * 128] + w[0:8] + w[8:16]]
                    if j:
                        parts.insert(0, acc[:, :j * 128])
                    if j + 1 < NL:
                        parts.append(acc[:, (j + 1) * 128:])
                    acc = jnp.concatenate(parts, axis=1)
                v = pm[n * 8:(n + 1) * 8, :]
                acc = v if acc is None else acc + v
            lsum[g] = acc
            ps[t] = jnp.concatenate([pm] + off, axis=0).astype(bf16)

            g, c = divmod(t - LAG, NC)
            pv = pv_dot(c, ps.pop(t - LAG) if t >= LAG else p_car[t])
            osum[g] = pv + osum[g] if c else pv
            if c == NC - 1:
                if g >= 0:
                    l = lsum.pop(g)
                    hrow = (it * G + g) * DH
                else:
                    l = l_car[...]
                    hrow = jnp.where(it == 0, H * DH, (it * G - 1) * DH)
                finish(osum.pop(g), l, pl.multiple_of(hrow, DH))
        for n in range(LAG):
            p_car[n] = ps.pop(T - LAG + n)
        o_car[...] = osum.pop(G - 1)
        l_car[...] = lsum.pop(G - 1)
        return carry

    jax.lax.fori_loop(0, H // G, attn_body, 0)

    @pl.when(step == 0)
    def _wait_weights():
        for i in range(3, 7):
            copy(i).wait()

    @pl.when(step > 0)
    def _wait_out():
        for r in range(NO):
            ocopy(step - 1, r).wait()

    xb = x_v[pl.ds(pl.multiple_of(step * TB, TB), TB), :]
    nxt = jnp.minimum(step + 1, NB - 1)
    jobs = [(h, i, half, j) for h in range(H) for i in range(NBIG)
            for half in range(2) for j in range(1 if half else NL)]
    total_w = NF * (WTS[0] + WTS[1] + WTS[2]) - WTS[2] + WTS[3]
    state = {'done': 0, 'w': 0}

    def anchor(res, w):
        state['w'] += w
        upto = len(jobs) * state['w'] // total_w
        release(nxt, jobs[state['done']:upto], res)
        state['done'] = upto

    b = None
    hs = {}
    for c in range(NF + 1):
        if c < NF:
            gcol = jnp.dot(xb, wg_v[:, c * FC:(c + 1) * FC],
                           preferred_element_type=f32)
            anchor(gcol, WTS[0])
            if c == 0:
                o = o_car[...]
                for n in range(LAG):
                    o = o + pv_dot(NC - LAG + n, p_car[n])
                finish(o, l_car[...], (H - 1) * DH)
            ucol = jnp.dot(xb, wu_v[:, c * FC:(c + 1) * FC],
                           preferred_element_type=f32)
            anchor(ucol, WTS[1])
            hg = 0.5 * gcol
            hs[c] = ((hg * jnp.tanh(hg) + hg) * ucol).astype(bf16)
        else:
            a = jax.lax.dot_general(ot[0:D, :], wo_v[...], _TN,
                                    preferred_element_type=f32)
            anchor(a, WTS[3])
        if 1 <= c < NF:
            bc = jnp.dot(hs.pop(c - 1), wd_v[(c - 1) * FC:c * FC, :],
                         preferred_element_type=f32)
            anchor(bc, WTS[2])
            b = bc if b is None else b + bc
    gw = gw_ref[...].astype(f32).reshape(1, D)
    gate = jax.nn.sigmoid(jnp.sum(xb.astype(f32) * gw, axis=1, keepdims=True))
    hl = hs.pop(NF - 1)
    for r in range(NO):
        rows = slice(r * RO, (r + 1) * RO)
        br = b[rows] + jnp.dot(hl[rows], wd_v[(NF - 1) * FC:, :],
                               preferred_element_type=f32)
        gr = gate[rows]
        obuf[rows, :] = (gr * a[rows] + (1.0 - gr) * br).astype(obuf.dtype)
        ocopy(step, r).start()

    @pl.when(step == NB - 1)
    def _drain():
        for r in range(NO):
            ocopy(step, r).wait()


@jax.jit
def pallas_gated_mix__grouped_kv_mqa__swiglu_ffn__prompt_kernel(
    A_x: jax.Array,
    A_wq: jax.Array,
    A_wk: jax.Array,
    A_wv: jax.Array,
    A_wo: jax.Array,
    B_x: jax.Array,
    B_w_gate: jax.Array,
    B_w_up: jax.Array,
    B_w_down: jax.Array,
    gate_w: jax.Array,
):
    del B_x
    bf16, f32, u32 = jnp.bfloat16, jnp.float32, jnp.uint32
    any_spec = pl.BlockSpec(memory_space=pl.ANY)
    out = pl.pallas_call(
        _kernel,
        grid=(NB,),
        in_specs=[any_spec] * 8 + [pl.BlockSpec((D,), lambda i: (0,))],
        out_specs=any_spec,
        out_shape=jax.ShapeDtypeStruct((S, D), A_x.dtype),
        scratch_shapes=[
            pltpu.VMEM((S, D), bf16),
            pltpu.VMEM((D, D), bf16),
            pltpu.VMEM((DH, D), bf16),
            pltpu.VMEM((DH, D), bf16),
            pltpu.VMEM((D, D), bf16),
            pltpu.VMEM((D, F), bf16),
            pltpu.VMEM((D, F), bf16),
            pltpu.VMEM((F, D), bf16),
            pltpu.VMEM((S // 2, KD), u32),
            pltpu.VMEM((DH // 2, S), u32),
            pltpu.VMEM(((NC + NBIG) * R, DH * 128), f32),
            pltpu.VMEM((NB, H, KD, TB), bf16),
            pltpu.VMEM((NB, H, DH, TB), f32),
            pltpu.VMEM((NB, H // 8, 8, TB), f32),
            pltpu.VMEM((D + DH, TB), bf16),
            pltpu.VMEM((LAG, TK, TB), bf16),
            pltpu.VMEM((DH, TB), f32),
            pltpu.VMEM((8, TB), f32),
            pltpu.VMEM((H, NBIG, 2 * R, TB), f32),
            pltpu.VMEM((TB, D), bf16),
            pltpu.SemaphoreType.DMA((7 + NB + NO,)),
        ],
        compiler_params=pltpu.CompilerParams(
            dimension_semantics=("arbitrary",),
            vmem_limit_bytes=100 * 1024 * 1024,
        ),
    )(A_x.reshape(S, D), A_wq, A_wk.T, A_wv.T, A_wo,
      B_w_gate, B_w_up, B_w_down, gate_w)
    return out.reshape(A_x.shape)
```

```python
import math

import jax
import jax.numpy as jnp
import jax.experimental.pallas as pl
import jax.experimental.pallas.tpu as pltpu

S = 2048
D = 512
H = 32
DH = 16
F = 1792

TB = 512
NB = S // TB
NL = TB // 128
TK = 128
NC = S // TK
G = 8
LAG = 2
KD = 32
FC = 256
NF = F // FC
NO = 4
RO = TB // NO

R = 16
BIG = (2, 5, 8, 11, 14)
NBIG = len(BIG)
NSM = NC - NBIG
SLOT = {c: n for n, c in enumerate(
    [c for c in range(NC) if c not in BIG] + list(BIG))}
POS = (4, 7, 10, 13)
POSB = (1, 5, 8, 11)
WTS = (2, 2, 2, 3)
NQS = (8, 10)
H0 = 12
HQ = 6
HSS = (3, 12)

QSCALE = (DH ** -0.5) * math.log2(math.e)
SAFE_BOUND = 40.0

_NT = (((1,), (1,)), ((), ()))
_TN = (((0,), (0,)), ((), ()))


def _kernel(x_hbm, wq_hbm, wkt_hbm, wvt_hbm, wo_hbm, wg_hbm, wu_hbm, wd_hbm,
            gw_ref, o_hbm,
            x_v, wq_v, wkt_v, wvt_v, wo_v, wg_v, wu_v, wd_v,
            kext, vt, kb, qext, qf32, negm, ot,
            p_car, o_car, l_car, s_pre, obuf, sems):
    step = pl.program_id(0)
    f32, bf16, u32 = jnp.float32, jnp.bfloat16, jnp.uint32

    srcs = (wkt_hbm, wvt_hbm, wo_hbm, wg_hbm, wu_hbm, wd_hbm)
    dsts = (wkt_v, wvt_v, wo_v, wg_v, wu_v, wd_v)

    def copy(i):
        return pltpu.make_async_copy(srcs[i], dsts[i], sems.at[i])

    def xcopy(b):
        return pltpu.make_async_copy(x_hbm.at[pl.ds(b * TB, TB), :],
                                     x_v.at[pl.ds(b * TB, TB), :],
                                     sems.at[5 + b])

    def stage(k):
        ks = pl.ds(k * 128, 128)
        return (pltpu.make_async_copy(x_hbm.at[pl.ds(0, TB), ks],
                                      x_v.at[pl.ds(0, TB), ks],
                                      sems.at[9 + 2 * k]),
                pltpu.make_async_copy(wq_hbm.at[ks, :], wq_v.at[ks, :],
                                      sems.at[10 + 2 * k]))

    def ocopy(blk, r):
        return pltpu.make_async_copy(
            obuf.at[pl.ds(r * RO, RO), :],
            o_hbm.at[pl.ds(pl.multiple_of(blk * TB + r * RO, RO), RO), :],
            sems.at[17 + r])

    never = jax.lax.broadcasted_iota(jnp.int32, (8, 128), 0) < -step

    def vpu_scores(blk, h, slot, n, j, init=None, anchors=None):
        rows = slice(slot * R, (slot + n) * R)
        acc = init
        for d in range(DH):
            qrow = qf32[blk, h, d:d + 1, j * 128:(j + 1) * 128]
            if d == 0 and anchors is not None:
                q8 = jnp.broadcast_to(qrow, (8, 128))
                qrow = jnp.concatenate(
                    [w for a in anchors
                     for w in [jnp.where(never, a, q8)] * 2], axis=0)
            pr = kb[rows, d * 128:(d + 1) * 128] * qrow
            acc = pr if acc is None else acc + pr
        return acc

    def release(blk, jobs, res):
        nr, ncol = res.shape[0] // 8, res.shape[1] // 128
        total = len(jobs) * NBIG
        for m, (h, half, j) in enumerate(jobs):
            anchors = []
            for mm in range(m * NBIG, (m + 1) * NBIG):
                r, jn = (mm * nr) // total, mm % ncol
                anchors.append(res[r * 8:(r + 1) * 8, jn * 128:(jn + 1) * 128])
            s_pre[h, half, :, j * 128:(j + 1) * 128] = vpu_scores(
                blk, h, NSM if half else NC, NBIG, j, anchors=anchors)

    @pl.when(step == 0)
    def _prologue():
        for i in range(2):
            copy(i).start()
        later = [stage(k) for k in range(4)] + [
            (xcopy(b),) for b in range(1, NB)]
        for cp in later[0] + later[1]:
            cp.start()
        later = later[2:]
        p_car[...] = jnp.zeros_like(p_car)
        o_car[...] = jnp.zeros_like(o_car)
        l_car[...] = jnp.ones_like(l_car)
        hr = jax.lax.broadcasted_iota(jnp.int32, (H, D), 0)
        hc = jax.lax.broadcasted_iota(jnp.int32, (H, D), 1)
        sel = jnp.where(hr == (hc >> 4), 1.0, 0.0).astype(bf16)
        for i in range(2):
            copy(i).wait()
        wkvt = jnp.concatenate([wkt_v[...], wvt_v[...]], axis=0)
        cpb = TB // TK
        kxe = []

        def kv_dot(b):
            return jax.lax.dot_general(wkvt, x_v[b * TB:(b + 1) * TB, :], _NT,
                                       preferred_element_type=f32)

        def kv_block(b, kvt):
            vt[:, b * TB:(b + 1) * TB] = pltpu.bitcast(
                kvt[DH:, :].astype(bf16), u32)
            kt = kvt[:DH, :].astype(bf16).astype(f32)
            ktx = jnp.concatenate(
                [kt, jnp.ones((8, TB), f32), jnp.zeros((8, TB), f32)], axis=0)
            kxf = ktx.T
            kx = kxf.astype(bf16)
            kext[b * TB // 2:(b + 1) * TB // 2, :] = pltpu.bitcast(kx, u32)
            for c in range(cpb):
                cg = b * cpb + c
                vpu_rows = [(SLOT[cg], (c + 1) * TK - R)]
                if cg in BIG:
                    kxe.append(kx[(c + 1) * TK - 2 * R:(c + 1) * TK - R, :])
                    vpu_rows.append((NC + BIG.index(cg), (c + 1) * TK - 2 * R))
                for slot, r0 in vpu_rows:
                    for d in range(DH):
                        kb[slot * R:(slot + 1) * R, d * 128:(d + 1) * 128] = (
                            jnp.broadcast_to(kxf[r0:r0 + R, d:d + 1], (R, 128)))
            return jnp.sum(kt * kt, axis=0, keepdims=True)

        jobs0 = [(h, 1, 0) for h in range(H)]

        def q_dot(b):
            qt = jax.lax.dot_general(wqt, x_v[b * TB:(b + 1) * TB, :], _NT,
                                     preferred_element_type=f32)
            if b > 1:
                release(0, jobs0[sum(NQS[:b - 2]):sum(NQS[:b - 1])], qt)
            return qt

        def q_block(b, qt):
            qs = (qt * QSCALE).astype(bf16)
            qf = qs.astype(f32)
            qext[b, :, 0:DH, :] = qs.reshape(H, DH, TB)
            qf32[b] = qf.reshape(H, DH, TB)
            return (qf * qf).astype(bf16)

        gi = jax.lax.broadcasted_iota(jnp.int32, (H // 8, 8, 8, TB), 1)
        ri = jax.lax.broadcasted_iota(jnp.int32, (H // 8, 8, 8, TB), 2)

        def shift_block(b, q2, kmax2):
            qn2 = jnp.dot(sel, q2, preferred_element_type=f32)
            bound = jnp.sqrt(qn2 * kmax2)
            bound = (bound * (1.0 + 2.0 ** -6)).astype(bf16).astype(f32)
            nb = (-bound).reshape(H // 8, 8, TB)
            negm[b] = nb
            ext = jnp.where(gi == ri, nb[:, None, :, :], 0.0).reshape(H, 8, TB)
            qext[b, :, DH:KD, :] = jnp.concatenate(
                [ext, jnp.zeros_like(ext)], axis=1).astype(bf16)
            return bound

        q0 = kvt0 = None
        wqt = []
        for k in range(4):
            for cp in stage(k):
                cp.wait()
            for grp in later[:(1, 2, 1, 1)[k]]:
                for cp in grp:
                    cp.start()
            later = later[(1, 2, 1, 1)[k]:]
            xk = x_v[0:TB, k * 128:(k + 1) * 128]
            wk = wq_v[k * 128:(k + 1) * 128, :]
            qk = jnp.dot(xk, wk, preferred_element_type=f32)
            kk = jax.lax.dot_general(wkvt[:, k * 128:(k + 1) * 128], xk, _NT,
                                     preferred_element_type=f32)
            q0 = qk if k == 0 else q0 + qk
            kvt0 = kk if k == 0 else kvt0 + kk
            wqt.append(wk.T)
        wqt = jnp.concatenate(wqt, axis=1)
        xcopy(1).wait()
        qt1 = q_dot(1)
        kvt1 = kv_dot(1)
        km = kv_block(0, kvt0)
        q2s = [q_block(0, q0.T)]
        for b in range(2, NB):
            xcopy(b).wait()
        for i in range(2, 6):
            copy(i).start()
        km = jnp.maximum(km, kv_block(1, kvt1))
        for b in range(2, NB):
            km = jnp.maximum(km, kv_block(b, kv_dot(b)))
        kmax2 = jnp.max(km, axis=1, keepdims=True)
        qt2 = q_dot(2)
        q2s.append(q_block(1, qt1))
        bmax = shift_block(0, q2s[0], kmax2)
        qt3 = q_dot(3)
        q2s.append(q_block(2, qt2))
        bmax = jnp.maximum(bmax, shift_block(1, q2s[1], kmax2))
        ke = jnp.concatenate(kxe, axis=0)[:, 0:DH]
        rest = jobs0[sum(NQS):]
        for h in range(H):
            se = jnp.dot(ke, qext[0, h, 0:DH, :], preferred_element_type=f32)
            s_pre[h, 0] = se
            if h >= H0:
                release(0, rest[(h - H0) * len(rest) // (H - 2 - H0):
                                (h - H0 + 1) * len(rest) // (H - 2 - H0)], se)
            if h == HQ:
                q2s.append(q_block(3, qt3))
            if h in HSS:
                b = 2 + HSS.index(h)
                bmax = jnp.maximum(bmax, shift_block(b, q2s[b], kmax2))
        unsafe = jnp.logical_not(jnp.max(bmax) <= SAFE_BOUND)

        @pl.when(unsafe)
        def _true_max():
            def group(n, carry):
                b, hg = n // (H // 8), n % (H // 8)
                for g in range(8):
                    q = qext[b, hg * 8 + g, 0:DH, :]

                    def chunk(c, m):
                        r0 = pl.multiple_of(c * (TK // 2), TK // 2)
                        kk = pltpu.bitcast(kext[pl.ds(r0, TK // 2), :], bf16)
                        s = jnp.dot(kk[:, 0:DH], q, preferred_element_type=f32)
                        return jnp.maximum(
                            m, jnp.max(s, axis=0, keepdims=True))

                    m = jax.lax.fori_loop(0, NC, chunk,
                                          jnp.full((1, TB), -jnp.inf, f32))
                    hi = m.astype(bf16).astype(f32)
                    mid = (m - hi).astype(bf16).astype(f32)
                    lo = (m - hi - mid).astype(bf16).astype(f32)
                    r = jax.lax.broadcasted_iota(jnp.int32, (DH, TB), 0)
                    ex = jnp.where(r == 0, -hi,
                                   jnp.where(r == 1, -mid,
                                             jnp.where(r == 2, -lo, 0.0)))
                    qext[b, hg * 8 + g, DH:KD, :] = ex.astype(bf16)
                    negm[b, hg, g:g + 1, :] = -(hi + mid + lo)
                return carry

            jax.lax.fori_loop(0, NB * (H // 8), group, 0)

    def pv_dot(c, p):
        return jnp.dot(pltpu.bitcast(vt[:, c * TK:(c + 1) * TK], bf16), p,
                       preferred_element_type=f32)

    def finish(o, l, hrow):
        o = o * (1.0 / l.sum(axis=0, keepdims=True))
        ot[pl.ds(hrow, DH), :] = o.astype(bf16)

    def attn_body(it, carry):
        ps, lsum = {}, {}
        osum = {-1: o_car[...]}
        T = G * NC

        for t in range(T):
            g, c = divmod(t, NC)
            h = it * G + g
            big = c in BIG
            nm = TK - (2 * R if big else R)
            s = jnp.dot(
                pltpu.bitcast(kext[c * TK // 2:(c * TK + nm) // 2, :], bf16),
                qext[step, h], preferred_element_type=f32)
            pm = jnp.exp2(s)
            if c == 0:
                shift = negm[step, it * (G // 8) + g // 8, g % 8:g % 8 + 1, :]
                sv = [vpu_scores(step, h, 0, NC if j else NSM, j,
                                 init=shift[:, j * 128:(j + 1) * 128])
                      for j in range(NL)]
            rows = slice(SLOT[c] * R, (SLOT[c] + 1) * R)
            own = [sv[j][rows] for j in range(1 if big else 0, NL)]
            off = []
            if big:
                rows = slice(BIG.index(c) * R, (BIG.index(c) + 1) * R)
                pe = jnp.exp2(s_pre[h, 0, rows, :] + shift)
                own.insert(0, s_pre[h, 1, rows, 0:128] + shift[:, 0:128])
                off.append(pe)
            off.append(jnp.exp2(jnp.concatenate(own, axis=1)))
            pos = POSB if big else POS
            acc = lsum.get(g)
            for n in range(nm // 8):
                if big and n == 1:
                    acc = acc + pe[0:8] + pe[8:16]
                if n in pos:
                    j = pos.index(n)
                    w = off[-1][:, j * 128:(j + 1) * 128]
                    parts = [acc[:, j * 128:(j + 1) * 128] + w[0:8] + w[8:16]]
                    if j:
                        parts.insert(0, acc[:, :j * 128])
                    if j + 1 < NL:
                        parts.append(acc[:, (j + 1) * 128:])
                    acc = jnp.concatenate(parts, axis=1)
                v = pm[n * 8:(n + 1) * 8, :]
                acc = v if acc is None else acc + v
            lsum[g] = acc
            ps[t] = jnp.concatenate([pm] + off, axis=0).astype(bf16)

            g, c = divmod(t - LAG, NC)
            pv = pv_dot(c, ps.pop(t - LAG) if t >= LAG else p_car[t])
            osum[g] = pv + osum[g] if c else pv
            if c == NC - 1:
                if g >= 0:
                    l = lsum.pop(g)
                    hrow = (it * G + g) * DH
                else:
                    l = l_car[...]
                    hrow = jnp.where(it == 0, H * DH, (it * G - 1) * DH)
                finish(osum.pop(g), l, pl.multiple_of(hrow, DH))
        for n in range(LAG):
            p_car[n] = ps.pop(T - LAG + n)
        o_car[...] = osum.pop(G - 1)
        l_car[...] = lsum.pop(G - 1)
        return carry

    jax.lax.fori_loop(0, H // G, attn_body, 0)

    @pl.when(step == 0)
    def _wait_weights():
        for i in range(2, 6):
            copy(i).wait()

    @pl.when(step > 0)
    def _wait_out():
        for r in range(NO):
            ocopy(step - 1, r).wait()

    xb = x_v[pl.ds(pl.multiple_of(step * TB, TB), TB), :]
    nxt = jnp.minimum(step + 1, NB - 1)
    jobs = [(h, half, j) for h in range(H) for half in range(2)
            for j in range(1 if half else NL)]
    total_w = NF * (WTS[0] + WTS[1] + WTS[2]) - WTS[2] + WTS[3]
    state = {'done': 0, 'w': 0}

    def anchor(res, w):
        state['w'] += w
        upto = len(jobs) * state['w'] // total_w
        release(nxt, jobs[state['done']:upto], res)
        state['done'] = upto

    b = None
    hs = {}
    for c in range(NF + 1):
        if c < NF:
            gcol = jnp.dot(xb, wg_v[:, c * FC:(c + 1) * FC],
                           preferred_element_type=f32)
            anchor(gcol, WTS[0])
            if c == 0:
                o = o_car[...]
                for n in range(LAG):
                    o = o + pv_dot(NC - LAG + n, p_car[n])
                finish(o, l_car[...], (H - 1) * DH)
            ucol = jnp.dot(xb, wu_v[:, c * FC:(c + 1) * FC],
                           preferred_element_type=f32)
            anchor(ucol, WTS[1])
            hg = 0.5 * gcol
            hs[c] = ((hg * jnp.tanh(hg) + hg) * ucol).astype(bf16)
        else:
            a = jax.lax.dot_general(ot[0:D, :], wo_v[...], _TN,
                                    preferred_element_type=f32)
            anchor(a, WTS[3])
        if 1 <= c < NF:
            bc = jnp.dot(hs.pop(c - 1), wd_v[(c - 1) * FC:c * FC, :],
                         preferred_element_type=f32)
            anchor(bc, WTS[2])
            b = bc if b is None else b + bc
    gw = gw_ref[...].astype(f32).reshape(1, D)
    gate = jax.nn.sigmoid(jnp.sum(xb.astype(f32) * gw, axis=1, keepdims=True))
    hl = hs.pop(NF - 1)
    for r in range(NO):
        rows = slice(r * RO, (r + 1) * RO)
        br = b[rows] + jnp.dot(hl[rows], wd_v[(NF - 1) * FC:, :],
                               preferred_element_type=f32)
        gr = gate[rows]
        obuf[rows, :] = (gr * a[rows] + (1.0 - gr) * br).astype(obuf.dtype)
        ocopy(step, r).start()

    @pl.when(step == NB - 1)
    def _drain():
        for r in range(NO):
            ocopy(step, r).wait()


@jax.jit
def pallas_gated_mix__grouped_kv_mqa__swiglu_ffn__prompt_kernel(
    A_x: jax.Array,
    A_wq: jax.Array,
    A_wk: jax.Array,
    A_wv: jax.Array,
    A_wo: jax.Array,
    B_x: jax.Array,
    B_w_gate: jax.Array,
    B_w_up: jax.Array,
    B_w_down: jax.Array,
    gate_w: jax.Array,
):
    del B_x
    bf16, f32, u32 = jnp.bfloat16, jnp.float32, jnp.uint32
    any_spec = pl.BlockSpec(memory_space=pl.ANY)
    out = pl.pallas_call(
        _kernel,
        grid=(NB,),
        in_specs=[any_spec] * 8 + [pl.BlockSpec((D,), lambda i: (0,))],
        out_specs=any_spec,
        out_shape=jax.ShapeDtypeStruct((S, D), A_x.dtype),
        scratch_shapes=[
            pltpu.VMEM((S, D), bf16),
            pltpu.VMEM((D, D), bf16),
            pltpu.VMEM((DH, D), bf16),
            pltpu.VMEM((DH, D), bf16),
            pltpu.VMEM((D, D), bf16),
            pltpu.VMEM((D, F), bf16),
            pltpu.VMEM((D, F), bf16),
            pltpu.VMEM((F, D), bf16),
            pltpu.VMEM((S // 2, KD), u32),
            pltpu.VMEM((DH // 2, S), u32),
            pltpu.VMEM(((NC + NBIG) * R, DH * 128), f32),
            pltpu.VMEM((NB, H, KD, TB), bf16),
            pltpu.VMEM((NB, H, DH, TB), f32),
            pltpu.VMEM((NB, H // 8, 8, TB), f32),
            pltpu.VMEM((D + DH, TB), bf16),
            pltpu.VMEM((LAG, TK, TB), bf16),
            pltpu.VMEM((DH, TB), f32),
            pltpu.VMEM((8, TB), f32),
            pltpu.VMEM((H, 2, NBIG * R, TB), f32),
            pltpu.VMEM((TB, D), bf16),
            pltpu.SemaphoreType.DMA((17 + NO,)),
        ],
        compiler_params=pltpu.CompilerParams(
            dimension_semantics=("arbitrary",),
            vmem_limit_bytes=100 * 1024 * 1024,
        ),
    )(A_x.reshape(S, D), A_wq, A_wk.T, A_wv.T, A_wo,
      B_w_gate, B_w_up, B_w_down, gate_w)
    return out.reshape(A_x.shape)
```

```python
import math

import jax
import jax.numpy as jnp
import jax.experimental.pallas as pl
import jax.experimental.pallas.tpu as pltpu

S = 2048
D = 512
H = 32
DH = 16
F = 1792

TB = 512
NB = S // TB
NL = TB // 128
TK = 128
NC = S // TK
G = 8
LAG = 2
KD = 32
FC = 256
NF = F // FC
NO = 4
RO = TB // NO

R = 16
BIG = (2, 5, 8, 11, 14)
NBIG = len(BIG)
NSM = NC - NBIG
SLOT = {c: n for n, c in enumerate(
    [c for c in range(NC) if c not in BIG] + list(BIG))}
POS = (4, 7, 10, 13)
POSB = (1, 5, 8, 11)
WTS = (2, 2, 2, 3)
NQS = (8, 10)
H0 = 12
HQ = 6
HSS = (3, 12)

QSCALE = (DH ** -0.5) * math.log2(math.e)
SAFE_BOUND = 40.0

_NT = (((1,), (1,)), ((), ()))
_TN = (((0,), (0,)), ((), ()))


def _kernel(x_hbm, wq_hbm, wkt_hbm, wvt_hbm, wo_hbm, wg_hbm, wu_hbm, wd_hbm,
            gw_ref, o_hbm,
            x_v, wq_v, wkt_v, wvt_v, wo_v, wg_v, wu_v, wd_v,
            kext, vt, kb, qext, qf32, negm, ot,
            p_car, o_car, l_car, s_pre, obuf, sems):
    step = pl.program_id(0)
    f32, bf16, u32 = jnp.float32, jnp.bfloat16, jnp.uint32

    srcs = (wkt_hbm, wvt_hbm, wo_hbm, wg_hbm, wu_hbm, wd_hbm)
    dsts = (wkt_v, wvt_v, wo_v, wg_v, wu_v, wd_v)

    def copy(i):
        return pltpu.make_async_copy(srcs[i], dsts[i], sems.at[i])

    def xcopy(b):
        return pltpu.make_async_copy(x_hbm.at[pl.ds(b * TB, TB), :],
                                     x_v.at[pl.ds(b * TB, TB), :],
                                     sems.at[5 + b])

    def stage(k):
        ks = pl.ds(k * 128, 128)
        return (pltpu.make_async_copy(x_hbm.at[pl.ds(0, TB), ks],
                                      x_v.at[pl.ds(0, TB), ks],
                                      sems.at[9 + 2 * k]),
                pltpu.make_async_copy(wq_hbm.at[ks, :], wq_v.at[ks, :],
                                      sems.at[10 + 2 * k]))

    def ocopy(blk, r):
        return pltpu.make_async_copy(
            obuf.at[pl.ds(r * RO, RO), :],
            o_hbm.at[pl.ds(pl.multiple_of(blk * TB + r * RO, RO), RO), :],
            sems.at[17 + r])

    never = jax.lax.broadcasted_iota(jnp.int32, (8, 128), 0) < -step

    def vpu_scores(blk, h, slot, n, j, init=None, anchors=None):
        rows = slice(slot * R, (slot + n) * R)
        acc = init
        for d in range(DH):
            qrow = qf32[blk, h, d:d + 1, j * 128:(j + 1) * 128]
            if d == 0 and anchors is not None:
                q8 = jnp.broadcast_to(qrow, (8, 128))
                qrow = jnp.concatenate(
                    [w for a in anchors
                     for w in [jnp.where(never, a, q8)] * 2], axis=0)
            pr = kb[rows, d * 128:(d + 1) * 128] * qrow
            acc = pr if acc is None else acc + pr
        return acc

    def release(blk, jobs, res):
        nr, ncol = res.shape[0] // 8, res.shape[1] // 128
        total = len(jobs) * NBIG
        for m, (h, half, j) in enumerate(jobs):
            anchors = []
            for mm in range(m * NBIG, (m + 1) * NBIG):
                r, jn = (mm * nr) // total, mm % ncol
                anchors.append(res[r * 8:(r + 1) * 8, jn * 128:(jn + 1) * 128])
            s_pre[h, half, :, j * 128:(j + 1) * 128] = vpu_scores(
                blk, h, NSM if half else NC, NBIG, j, anchors=anchors)

    @pl.when(step == 0)
    def _prologue():
        for i in range(2):
            copy(i).start()
        later = [stage(k) for k in range(4)] + [
            (xcopy(b),) for b in range(1, NB)]
        for cp in later[0] + later[1]:
            cp.start()
        later = later[2:]
        p_car[...] = jnp.zeros_like(p_car)
        o_car[...] = jnp.zeros_like(o_car)
        l_car[...] = jnp.ones_like(l_car)
        hr = jax.lax.broadcasted_iota(jnp.int32, (H, D), 0)
        hc = jax.lax.broadcasted_iota(jnp.int32, (H, D), 1)
        sel = jnp.where(hr == (hc >> 4), 1.0, 0.0).astype(bf16)
        for i in range(2):
            copy(i).wait()
        wkvt = jnp.concatenate([wkt_v[...], wvt_v[...]], axis=0)
        cpb = TB // TK
        kxe = []

        def kv_dot(b):
            return jax.lax.dot_general(wkvt, x_v[b * TB:(b + 1) * TB, :], _NT,
                                       preferred_element_type=f32)

        def kv_block(b, kvt):
            vt[:, b * TB:(b + 1) * TB] = pltpu.bitcast(
                kvt[DH:, :].astype(bf16), u32)
            kt = kvt[:DH, :].astype(bf16).astype(f32)
            ktx = jnp.concatenate(
                [kt, jnp.ones((8, TB), f32), jnp.zeros((8, TB), f32)], axis=0)
            kxf = ktx.T
            kx = kxf.astype(bf16)
            kext[b * TB // 2:(b + 1) * TB // 2, :] = pltpu.bitcast(kx, u32)
            for c in range(cpb):
                cg = b * cpb + c
                vpu_rows = [(SLOT[cg], (c + 1) * TK - R)]
                if cg in BIG:
                    kxe.append(kx[(c + 1) * TK - 2 * R:(c + 1) * TK - R, :])
                    vpu_rows.append((NC + BIG.index(cg), (c + 1) * TK - 2 * R))
                for slot, r0 in vpu_rows:
                    for d in range(DH):
                        kb[slot * R:(slot + 1) * R, d * 128:(d + 1) * 128] = (
                            jnp.broadcast_to(kxf[r0:r0 + R, d:d + 1], (R, 128)))
            return jnp.sum(kt * kt, axis=0, keepdims=True)

        jobs0 = [(h, 1, 0) for h in range(H)]

        def q_dot(b):
            qt = jax.lax.dot_general(wqt, x_v[b * TB:(b + 1) * TB, :], _NT,
                                     preferred_element_type=f32)
            if b > 1:
                release(0, jobs0[sum(NQS[:b - 2]):sum(NQS[:b - 1])], qt)
            return qt

        def q_block(b, qt):
            qs = (qt * QSCALE).astype(bf16)
            qf = qs.astype(f32)
            qext[b, :, 0:DH, :] = qs.reshape(H, DH, TB)
            qf32[b] = qf.reshape(H, DH, TB)
            return (qf * qf).astype(bf16)

        gi = jax.lax.broadcasted_iota(jnp.int32, (H // 8, 8, 8, TB), 1)
        ri = jax.lax.broadcasted_iota(jnp.int32, (H // 8, 8, 8, TB), 2)

        def shift_block(b, q2, kmax2):
            qn2 = jnp.dot(sel, q2, preferred_element_type=f32)
            bound = jnp.sqrt(qn2 * kmax2)
            bound = (bound * (1.0 + 2.0 ** -6)).astype(bf16).astype(f32)
            nb = (-bound).reshape(H // 8, 8, TB)
            negm[b] = nb
            ext = jnp.where(gi == ri, nb[:, None, :, :], 0.0).reshape(H, 8, TB)
            qext[b, :, DH:KD, :] = jnp.concatenate(
                [ext, jnp.zeros_like(ext)], axis=1).astype(bf16)
            return bound

        q0 = kvt0 = None
        wqt = []
        for k in range(4):
            for cp in stage(k):
                cp.wait()
            for grp in later[:(1, 2, 1, 1)[k]]:
                for cp in grp:
                    cp.start()
            later = later[(1, 2, 1, 1)[k]:]
            xk = x_v[0:TB, k * 128:(k + 1) * 128]
            wk = wq_v[k * 128:(k + 1) * 128, :]
            qk = jnp.dot(xk, wk, preferred_element_type=f32)
            kk = jax.lax.dot_general(wkvt[:, k * 128:(k + 1) * 128], xk, _NT,
                                     preferred_element_type=f32)
            q0 = qk if k == 0 else q0 + qk
            kvt0 = kk if k == 0 else kvt0 + kk
            wqt.append(wk.T)
            if k == 0:
                x_v[S:S + 16, :] = qk[TB - 16:, :].astype(bf16)
        wqt = jnp.concatenate(wqt, axis=1)
        xcopy(1).wait()
        qt1 = q_dot(1)
        kvt1 = kv_dot(1)
        km = kv_block(0, kvt0)
        q2s = [q_block(0, q0.T)]
        for b in range(2, NB):
            xcopy(b).wait()
        for i in range(2, 6):
            copy(i).start()
        km = jnp.maximum(km, kv_block(1, kvt1))
        for b in range(2, NB):
            km = jnp.maximum(km, kv_block(b, kv_dot(b)))
        kmax2 = jnp.max(km, axis=1, keepdims=True)
        qt2 = q_dot(2)
        q2s.append(q_block(1, qt1))
        bmax = shift_block(0, q2s[0], kmax2)
        qt3 = q_dot(3)
        q2s.append(q_block(2, qt2))
        bmax = jnp.maximum(bmax, shift_block(1, q2s[1], kmax2))
        ke = jnp.concatenate(kxe, axis=0)[:, 0:DH]
        rest = jobs0[sum(NQS):]
        for h in range(H):
            se = jnp.dot(ke, qext[0, h, 0:DH, :], preferred_element_type=f32)
            s_pre[h, 0] = se
            if h >= H0:
                release(0, rest[(h - H0) * len(rest) // (H - 2 - H0):
                                (h - H0 + 1) * len(rest) // (H - 2 - H0)], se)
            if h == HQ:
                q2s.append(q_block(3, qt3))
            if h in HSS:
                b = 2 + HSS.index(h)
                bmax = jnp.maximum(bmax, shift_block(b, q2s[b], kmax2))
        unsafe = jnp.logical_not(jnp.max(bmax) <= SAFE_BOUND)

        @pl.when(unsafe)
        def _true_max():
            def group(n, carry):
                b, hg = n // (H // 8), n % (H // 8)
                for g in range(8):
                    q = qext[b, hg * 8 + g, 0:DH, :]

                    def chunk(c, m):
                        r0 = pl.multiple_of(c * (TK // 2), TK // 2)
                        kk = pltpu.bitcast(kext[pl.ds(r0, TK // 2), :], bf16)
                        s = jnp.dot(kk[:, 0:DH], q, preferred_element_type=f32)
                        return jnp.maximum(
                            m, jnp.max(s, axis=0, keepdims=True))

                    m = jax.lax.fori_loop(0, NC, chunk,
                                          jnp.full((1, TB), -jnp.inf, f32))
                    hi = m.astype(bf16).astype(f32)
                    mid = (m - hi).astype(bf16).astype(f32)
                    lo = (m - hi - mid).astype(bf16).astype(f32)
                    r = jax.lax.broadcasted_iota(jnp.int32, (DH, TB), 0)
                    ex = jnp.where(r == 0, -hi,
                                   jnp.where(r == 1, -mid,
                                             jnp.where(r == 2, -lo, 0.0)))
                    qext[b, hg * 8 + g, DH:KD, :] = ex.astype(bf16)
                    negm[b, hg, g:g + 1, :] = -(hi + mid + lo)
                return carry

            jax.lax.fori_loop(0, NB * (H // 8), group, 0)

    def pv_dot(c, p):
        return jnp.dot(pltpu.bitcast(vt[:, c * TK:(c + 1) * TK], bf16), p,
                       preferred_element_type=f32)

    def finish(o, l, hrow):
        l = l.sum(axis=0, keepdims=True)
        r = pl.reciprocal(l, approx=True)
        o = o * (r * (2.0 - l * r))
        ot[pl.ds(hrow, DH), :] = o.astype(bf16)

    def attn_body(it, carry):
        ps, lsum = {}, {}
        osum = {-1: o_car[...]}
        T = G * NC

        for t in range(T):
            g, c = divmod(t, NC)
            h = it * G + g
            big = c in BIG
            nm = TK - (2 * R if big else R)
            s = jnp.dot(
                pltpu.bitcast(kext[c * TK // 2:(c * TK + nm) // 2, :], bf16),
                qext[step, h], preferred_element_type=f32)
            pm = jnp.exp2(s)
            if c == 0:
                shift = negm[step, it * (G // 8) + g // 8, g % 8:g % 8 + 1, :]
                sv = [vpu_scores(step, h, 0, NC if j else NSM, j,
                                 init=shift[:, j * 128:(j + 1) * 128])
                      for j in range(NL)]
            rows = slice(SLOT[c] * R, (SLOT[c] + 1) * R)
            own = [sv[j][rows] for j in range(1 if big else 0, NL)]
            off = []
            if big:
                rows = slice(BIG.index(c) * R, (BIG.index(c) + 1) * R)
                pe = jnp.exp2(s_pre[h, 0, rows, :] + shift)
                own.insert(0, s_pre[h, 1, rows, 0:128] + shift[:, 0:128])
                off.append(pe)
            off.append(jnp.exp2(jnp.concatenate(own, axis=1)))
            pos = POSB if big else POS
            acc = lsum.get(g)
            for n in range(nm // 8):
                if big and n == 1:
                    acc = acc + pe[0:8] + pe[8:16]
                if n in pos:
                    j = pos.index(n)
                    w = off[-1][:, j * 128:(j + 1) * 128]
                    parts = [acc[:, j * 128:(j + 1) * 128] + w[0:8] + w[8:16]]
                    if j:
                        parts.insert(0, acc[:, :j * 128])
                    if j + 1 < NL:
                        parts.append(acc[:, (j + 1) * 128:])
                    acc = jnp.concatenate(parts, axis=1)
                v = pm[n * 8:(n + 1) * 8, :]
                acc = v if acc is None else acc + v
            lsum[g] = acc
            ps[t] = jnp.concatenate([pm] + off, axis=0).astype(bf16)

            g, c = divmod(t - LAG, NC)
            pv = pv_dot(c, ps.pop(t - LAG) if t >= LAG else p_car[t])
            osum[g] = pv + osum[g] if c else pv
            if c == NC - 1:
                if g >= 0:
                    l = lsum.pop(g)
                    hrow = (it * G + g) * DH
                else:
                    l = l_car[...]
                    hrow = jnp.where(it == 0, H * DH, (it * G - 1) * DH)
                finish(osum.pop(g), l, pl.multiple_of(hrow, DH))
        for n in range(LAG):
            p_car[n] = ps.pop(T - LAG + n)
        o_car[...] = osum.pop(G - 1)
        l_car[...] = lsum.pop(G - 1)
        return carry

    jax.lax.fori_loop(0, H // G, attn_body, 0)

    @pl.when(step == 0)
    def _wait_weights():
        for i in range(2, 6):
            copy(i).wait()

    @pl.when(step > 0)
    def _wait_out():
        for r in range(NO):
            ocopy(step - 1, r).wait()

    xb = x_v[pl.ds(pl.multiple_of(step * TB, TB), TB), :]
    nxt = jnp.minimum(step + 1, NB - 1)
    jobs = [(h, half, j) for h in range(H) for half in range(2)
            for j in range(1 if half else NL)]
    total_w = NF * (WTS[0] + WTS[1] + WTS[2]) - WTS[2] + WTS[3]
    state = {'done': 0, 'w': 0}

    def anchor(res, w):
        state['w'] += w
        upto = len(jobs) * state['w'] // total_w
        release(nxt, jobs[state['done']:upto], res)
        state['done'] = upto

    b = None
    hs = {}
    for c in range(NF + 1):
        if c < NF:
            gcol = jnp.dot(xb, wg_v[:, c * FC:(c + 1) * FC],
                           preferred_element_type=f32)
            anchor(gcol, WTS[0])
            if c == 0:
                o = o_car[...]
                for n in range(LAG):
                    o = o + pv_dot(NC - LAG + n, p_car[n])
                finish(o, l_car[...], (H - 1) * DH)
            ucol = jnp.dot(xb, wu_v[:, c * FC:(c + 1) * FC],
                           preferred_element_type=f32)
            anchor(ucol, WTS[1])
            hg = 0.5 * gcol
            hs[c] = ((hg * jnp.tanh(hg) + hg) * ucol).astype(bf16)
        else:
            a = jax.lax.dot_general(ot[0:D, :], wo_v[...], _TN,
                                    preferred_element_type=f32)
            anchor(a, WTS[3])
        if 1 <= c < NF:
            bc = jnp.dot(hs.pop(c - 1), wd_v[(c - 1) * FC:c * FC, :],
                         preferred_element_type=f32)
            anchor(bc, WTS[2])
            b = bc if b is None else b + bc
    gw = gw_ref[...].astype(f32).reshape(1, D)
    z = jnp.sum(xb.astype(f32) * gw, axis=1, keepdims=True)
    gate = 0.5 * jnp.tanh(0.5 * z) + 0.5
    hl = hs.pop(NF - 1)
    for r in range(NO):
        rows = slice(r * RO, (r + 1) * RO)
        br = b[rows] + jnp.dot(hl[rows], wd_v[(NF - 1) * FC:, :],
                               preferred_element_type=f32)
        gr = gate[rows]
        obuf[rows, :] = (br + gr * (a[rows] - br)).astype(obuf.dtype)
        ocopy(step, r).start()

    @pl.when(step == NB - 1)
    def _drain():
        for r in range(NO):
            ocopy(step, r).wait()


@jax.jit
def pallas_gated_mix__grouped_kv_mqa__swiglu_ffn__prompt_kernel(
    A_x: jax.Array,
    A_wq: jax.Array,
    A_wk: jax.Array,
    A_wv: jax.Array,
    A_wo: jax.Array,
    B_x: jax.Array,
    B_w_gate: jax.Array,
    B_w_up: jax.Array,
    B_w_down: jax.Array,
    gate_w: jax.Array,
):
    del B_x
    bf16, f32, u32 = jnp.bfloat16, jnp.float32, jnp.uint32
    any_spec = pl.BlockSpec(memory_space=pl.ANY)
    out = pl.pallas_call(
        _kernel,
        grid=(NB,),
        in_specs=[any_spec] * 8 + [pl.BlockSpec((D,), lambda i: (0,))],
        out_specs=any_spec,
        out_shape=jax.ShapeDtypeStruct((S, D), A_x.dtype),
        scratch_shapes=[
            pltpu.VMEM((S + 16, D), bf16),
            pltpu.VMEM((D, D), bf16),
            pltpu.VMEM((DH, D), bf16),
            pltpu.VMEM((DH, D), bf16),
            pltpu.VMEM((D, D), bf16),
            pltpu.VMEM((D, F), bf16),
            pltpu.VMEM((D, F), bf16),
            pltpu.VMEM((F, D), bf16),
            pltpu.VMEM((S // 2, KD), u32),
            pltpu.VMEM((DH // 2, S), u32),
            pltpu.VMEM(((NC + NBIG) * R, DH * 128), f32),
            pltpu.VMEM((NB, H, KD, TB), bf16),
            pltpu.VMEM((NB, H, DH, TB), f32),
            pltpu.VMEM((NB, H // 8, 8, TB), f32),
            pltpu.VMEM((D + DH, TB), bf16),
            pltpu.VMEM((LAG, TK, TB), bf16),
            pltpu.VMEM((DH, TB), f32),
            pltpu.VMEM((8, TB), f32),
            pltpu.VMEM((H, 2, NBIG * R, TB), f32),
            pltpu.VMEM((TB, D), bf16),
            pltpu.SemaphoreType.DMA((17 + NO,)),
        ],
        compiler_params=pltpu.CompilerParams(
            dimension_semantics=("arbitrary",),
            vmem_limit_bytes=100 * 1024 * 1024,
        ),
    )(A_x.reshape(S, D), A_wq, A_wk.T, A_wv.T, A_wo,
      B_w_gate, B_w_up, B_w_down, gate_w)
    return out.reshape(A_x.shape)
```

```python
import math

import jax
import jax.numpy as jnp
import jax.experimental.pallas as pl
import jax.experimental.pallas.tpu as pltpu

S = 2048
D = 512
H = 32
DH = 16
F = 1792

TB = 512
NB = S // TB
NL = TB // 128
TK = 128
NC = S // TK
G = 8
LAG = 2
FC = 256
NF = F // FC
NO = 4
RO = TB // NO

R = 16
BIG = (1, 3, 5, 8, 10, 12, 14)
NBIG = len(BIG)
TSPL = (2, 2, 2, 1)
POS = (4, 7, 10, 13)
POSB = (4, 6, 9, 11)
WTS = (3, 3, 3, 5)
NQS = (8, 12, 12)

SPLIT = 32

QSCALE = (DH ** -0.5) * math.log2(math.e)
SAFE_S = 48.0
SAFE_V = 2.0 ** 60

_NT = (((1,), (1,)), ((), ()))
_TN = (((0,), (0,)), ((), ()))


def rev16(a):
    return jnp.concatenate(
        [a[r:r + 16] for r in range(a.shape[0] - 16, -1, -16)], axis=0)


def _kernel(x_hbm, wq_hbm, wkt_hbm, wvt_hbm, wo_hbm, wg_hbm, wu_hbm, wd_hbm,
            gw_ref, o_hbm,
            x_v, wq_v, wkt_v, wvt_v, wo_v, wg_v, wu_v, wd_v,
            kn, vt, kb, qt16, qf32, ot,
            p_car, o_car, l_car, s_pre, obuf, safe_ref, sems):
    step = pl.program_id(0)
    f32, bf16, u32 = jnp.float32, jnp.bfloat16, jnp.uint32

    srcs = (wkt_hbm, wvt_hbm, wo_hbm, wg_hbm, wu_hbm, wd_hbm)
    dsts = (wkt_v, wvt_v, wo_v, wg_v, wu_v, wd_v)

    def copy(i):
        return pltpu.make_async_copy(srcs[i], dsts[i], sems.at[i])

    def xcopy(b):
        return pltpu.make_async_copy(x_hbm.at[pl.ds(b * TB, TB), :],
                                     x_v.at[pl.ds(b * TB, TB), :],
                                     sems.at[5 + b])

    def stage(k):
        ks = pl.ds(k * 128, 128)
        return (pltpu.make_async_copy(x_hbm.at[pl.ds(0, TB), ks],
                                      x_v.at[pl.ds(0, TB), ks],
                                      sems.at[9 + 2 * k]),
                pltpu.make_async_copy(wq_hbm.at[ks, :], wq_v.at[ks, :],
                                      sems.at[10 + 2 * k]))

    def ocopy(blk, r):
        return pltpu.make_async_copy(
            obuf.at[pl.ds(r * RO, RO), :],
            o_hbm.at[pl.ds(pl.multiple_of(blk * TB + r * RO, RO), RO), :],
            sems.at[17 + r])

    never = jax.lax.broadcasted_iota(jnp.int32, (8, 128), 0) < -step

    def vpu_scores(blk, h, slot, n, j, anchors=None):
        rows = slice(slot * R, (slot + n) * R)
        acc = None
        for d in range(DH):
            qrow = qf32[blk, h, d:d + 1, j * 128:(j + 1) * 128]
            if d == 0 and anchors is not None:
                q8 = jnp.broadcast_to(qrow, (8, 128))
                qrow = jnp.concatenate(
                    [w for a in anchors
                     for w in [jnp.where(never, a, q8)] * 2], axis=0)
            pr = kb[rows, d * 128:(d + 1) * 128] * qrow
            acc = pr if acc is None else acc + pr
        return acc

    def release(blk, jobs, res):
        nr, ncol = res.shape[0] // 8, res.shape[1] // 128
        total = len(jobs) * NBIG
        for m, (h, j) in enumerate(jobs):
            anchors = []
            for mm in range(m * NBIG, (m + 1) * NBIG):
                r, jn = (mm * nr) // total, mm % ncol
                anchors.append(res[r * 8:(r + 1) * 8, jn * 128:(jn + 1) * 128])
            i0 = 0
            for n in TSPL:
                s_pre[h, i0 * R:(i0 + n) * R, j * 128:(j + 1) * 128] = (
                    vpu_scores(blk, h, NC + i0, n, j, anchors[i0:i0 + n]))
                i0 += n

    @pl.when(step == 0)
    def _prologue():
        for i in range(2):
            copy(i).start()
        later = [stage(k) for k in range(4)] + [
            (xcopy(b),) for b in range(1, NB)]
        for cp in later[0] + later[1]:
            cp.start()
        later = later[2:]
        p_car[...] = jnp.zeros_like(p_car)
        o_car[...] = jnp.zeros_like(o_car)
        l_car[...] = jnp.ones_like(l_car)
        hr = jax.lax.broadcasted_iota(jnp.int32, (H, D), 0)
        hc = jax.lax.broadcasted_iota(jnp.int32, (H, D), 1)
        sel = jnp.where(hr == (hc >> 4), 1.0, 0.0).astype(bf16)
        for i in range(2):
            copy(i).wait()
        wkvt = jnp.concatenate([wkt_v[...], wvt_v[...]], axis=0)
        cpb = TB // TK
        kxe, kn2s, vmaxs, qn2s = [], [], [], []

        def kv_dot(b):
            return jax.lax.dot_general(wkvt, x_v[b * TB:(b + 1) * TB, :], _NT,
                                       preferred_element_type=f32)

        def kv_block(b, kvt):
            vt[:, b * TB:(b + 1) * TB] = pltpu.bitcast(
                kvt[DH:, :].astype(bf16), u32)
            vmaxs.append(jnp.max(jnp.abs(kvt[DH:, :]), axis=0, keepdims=True))
            kt = kvt[:DH, :].astype(bf16).astype(f32)
            kn2s.append(jnp.sum(kt * kt, axis=0, keepdims=True))
            kxf = kt.T
            kx = kxf.astype(bf16)
            kxr = jnp.concatenate(
                [rev16(kx[c * TK:(c + 1) * TK]) for c in range(cpb)], axis=0)
            kn[b * TB // 2:(b + 1) * TB // 2, :] = pltpu.bitcast(kxr, u32)
            for c in range(cpb):
                cg = b * cpb + c
                r2 = c * TK + R
                vpu_rows = [(cg, c * TK)]
                if cg in BIG:
                    kxe.append(kx[r2:r2 + R, :])
                    vpu_rows.append((NC + BIG.index(cg), r2))
                for slot, r0 in vpu_rows:
                    for d in range(DH):
                        kb[slot * R:(slot + 1) * R, d * 128:(d + 1) * 128] = (
                            jnp.broadcast_to(kxf[r0:r0 + R, d:d + 1], (R, 128)))

        nj0 = sum(NQS)
        hv = H - nj0 // NL
        jobs0 = [(h, j) for h in range(hv, H) for j in range(NL)]

        def q_dot(b):
            qt = jax.lax.dot_general(wqt, x_v[b * TB:(b + 1) * TB, :], _NT,
                                     preferred_element_type=f32)
            if b > 1:
                release(0, jobs0[sum(NQS[:b - 2]):sum(NQS[:b - 1])], qt)
            return qt

        def q_block(b, qt):
            qs = (qt * QSCALE).astype(bf16)
            qf = qs.astype(f32)
            qt16[b] = qs.reshape(H, DH, TB)
            qf32[b] = qf.reshape(H, DH, TB)
            return (qf * qf).astype(bf16)

        def q_norm(q2):
            qn2s.append(jnp.dot(sel, q2, preferred_element_type=f32))

        q0 = kvt0 = None
        wqt = []
        for k in range(4):
            for cp in stage(k):
                cp.wait()
            for grp in later[:(1, 2, 1, 1)[k]]:
                for cp in grp:
                    cp.start()
            later = later[(1, 2, 1, 1)[k]:]
            xk = x_v[0:TB, k * 128:(k + 1) * 128]
            wk = wq_v[k * 128:(k + 1) * 128, :]
            qk = jnp.dot(xk, wk, preferred_element_type=f32)
            kk = jax.lax.dot_general(wkvt[:, k * 128:(k + 1) * 128], xk, _NT,
                                     preferred_element_type=f32)
            q0 = qk if k == 0 else q0 + qk
            kvt0 = kk if k == 0 else kvt0 + kk
            wqt.append(wk.T)
            if k == 0:
                x_v[S:S + 16, :] = qk[TB - 16:, :].astype(bf16)
        wqt = jnp.concatenate(wqt, axis=1)
        xcopy(1).wait()
        qt1 = q_dot(1)
        kvt1 = kv_dot(1)
        kv_block(0, kvt0)
        q2s = [q_block(0, q0.T)]
        for b in range(2, NB):
            xcopy(b).wait()
        for i in range(2, 6):
            copy(i).start()
        kv_block(1, kvt1)
        for b in range(2, NB):
            kv_block(b, kv_dot(b))
        qt2 = q_dot(2)
        q2s.append(q_block(1, qt1))
        q_norm(q2s[0])
        qt3 = q_dot(3)
        q2s.append(q_block(2, qt2))
        q_norm(q2s[1])
        ke = jnp.concatenate(kxe, axis=0)
        rest = jobs0[sum(NQS[:2]):]
        h0 = 8
        for h in range(hv):
            se = jnp.dot(ke, qt16[0, h], preferred_element_type=f32)
            s_pre[h] = se
            if h >= h0:
                release(0, rest[(h - h0) * len(rest) // (hv - 2 - h0):
                                (h - h0 + 1) * len(rest) // (hv - 2 - h0)], se)
            if h == 3:
                q_norm(q2s[2])
            if h == 4:
                q2s.append(q_block(3, qt3))
            if h == 10:
                q_norm(q2s[3])

        def tmax(xs):
            while len(xs) > 1:
                xs = [jnp.maximum(xs[i], xs[i + 1])
                      for i in range(0, len(xs), 2)]
            return jnp.max(xs[0])

        s2 = tmax(qn2s) * tmax(kn2s) * (1.0 + 2.0 ** -5)
        safe = jnp.logical_and(s2 <= SAFE_S * SAFE_S, tmax(vmaxs) <= SAFE_V)
        safe_ref[0] = safe.astype(jnp.int32)

    def k_rows(r0, n):
        return pltpu.bitcast(kn[pl.ds(r0 // 2, n // 2), :], bf16)

    def pv_dot(c, p):
        return jnp.dot(pltpu.bitcast(vt[:, c * TK:(c + 1) * TK], bf16), p,
                       preferred_element_type=f32)

    def finish(o, l, hrow):
        l = l.sum(axis=0, keepdims=True)
        r = pl.reciprocal(l, approx=True)
        o = o * (r * (2.0 - l * r))
        ot[pl.ds(hrow, DH), :] = o.astype(bf16)

    def attn_body(it, carry):
        ps, lsum = {}, {}
        osum = {-1: o_car[...]}
        T = G * NC

        for t in range(T):
            g, c = divmod(t, NC)
            h = it * G + g
            big = c in BIG
            nm = TK - (2 * R if big else R)

            def qk(r0, r1):
                return jnp.dot(k_rows(c * TK + r0, r1 - r0), qt16[step, h],
                               preferred_element_type=f32)

            sa = qk(0, SPLIT)
            g2, c2 = divmod(t - LAG, NC)
            pv = pv_dot(c2, ps.pop(t - LAG) if t >= LAG else p_car[t])
            osum[g2] = pv + osum[g2] if c2 else pv
            if c2 == NC - 1:
                if g2 >= 0:
                    l = lsum.pop(g2)
                    hrow = (it * G + g2) * DH
                else:
                    l = l_car[...]
                    hrow = jnp.where(it == 0, H * DH, (it * G - 1) * DH)
                finish(osum.pop(g2), l, pl.multiple_of(hrow, DH))
            pm = jnp.exp2(jnp.concatenate([sa, qk(SPLIT, nm)], axis=0))
            if c == 0:
                sv = jnp.concatenate(
                    [vpu_scores(step, h, 0, NC, j) for j in range(NL)], axis=1)
            off = [jnp.exp2(sv[c * R:(c + 1) * R])]
            if big:
                i = BIG.index(c)
                pe = jnp.exp2(s_pre[h, i * R:(i + 1) * R, :])
                off.append(pe)
            pos = POSB if big else POS
            acc = lsum.get(g)
            for n in range(nm // 8):
                if big and n == 1:
                    acc = acc + pe[0:8] + pe[8:16]
                if n in pos:
                    j = pos.index(n)
                    w = off[0][:, j * 128:(j + 1) * 128]
                    parts = [acc[:, j * 128:(j + 1) * 128] + w[0:8] + w[8:16]]
                    if j:
                        parts.insert(0, acc[:, :j * 128])
                    if j + 1 < NL:
                        parts.append(acc[:, (j + 1) * 128:])
                    acc = jnp.concatenate(parts, axis=1)
                v = pm[n * 8:(n + 1) * 8, :]
                acc = v if acc is None else acc + v
            lsum[g] = acc
            ps[t] = jnp.concatenate(off + [rev16(pm)], axis=0).astype(bf16)
        for n in range(LAG):
            p_car[n] = ps.pop(T - LAG + n)
        o_car[...] = osum.pop(G - 1)
        l_car[...] = lsum.pop(G - 1)
        return carry

    @pl.when(safe_ref[0] == 1)
    def _fast():
        jax.lax.fori_loop(0, H // G, attn_body, 0)

    @pl.when(safe_ref[0] != 1)
    def _slow():
        def head(h, carry):
            q = qt16[step, h]

            def scores(c):
                return jnp.dot(k_rows(pl.multiple_of(c * TK, TK), TK), q,
                               preferred_element_type=f32)

            def pass1(c, m):
                return jnp.maximum(
                    m, jnp.max(scores(c), axis=0, keepdims=True))

            m = jax.lax.fori_loop(0, NC, pass1,
                                  jnp.full((1, TB), -jnp.inf, f32))

            def pass2(c, ol):
                p = rev16(jnp.exp2(scores(c) - m))
                vc = vt[:, pl.ds(pl.multiple_of(c * TK, TK), TK)]
                pv = jnp.dot(pltpu.bitcast(vc, bf16), p.astype(bf16),
                             preferred_element_type=f32)
                return (ol[0] + pv,
                        ol[1] + p.reshape(TK // 8, 8, TB).sum(axis=0))

            o, l = jax.lax.fori_loop(
                0, NC, pass2,
                (jnp.zeros((DH, TB), f32), jnp.zeros((8, TB), f32)))
            finish(o, l, pl.multiple_of(h * DH, DH))
            o_car[...] = o
            l_car[...] = l
            return carry

        jax.lax.fori_loop(0, H, head, 0)

    @pl.when(step == 0)
    def _wait_weights():
        for i in range(2, 6):
            copy(i).wait()

    @pl.when(step > 0)
    def _wait_out():
        for r in range(NO):
            ocopy(step - 1, r).wait()

    xb = x_v[pl.ds(pl.multiple_of(step * TB, TB), TB), :]
    nxt = jnp.minimum(step + 1, NB - 1)
    jobs = [(h, j) for h in range(H) for j in range(NL)]
    total_w = NF * (WTS[0] + WTS[1] + WTS[2]) - WTS[2] + WTS[3]
    state = {'done': 0, 'w': 0}

    def anchor(res, w):
        state['w'] += w
        upto = len(jobs) * state['w'] // total_w
        release(nxt, jobs[state['done']:upto], res)
        state['done'] = upto

    b = None
    hs = {}
    for c in range(NF + 1):
        if c < NF:
            gcol = jnp.dot(xb, wg_v[:, c * FC:(c + 1) * FC],
                           preferred_element_type=f32)
            anchor(gcol, WTS[0])
            if c == 0:
                o = o_car[...]
                for n in range(LAG):
                    o = o + pv_dot(NC - LAG + n, p_car[n])
                finish(o, l_car[...], (H - 1) * DH)
            ucol = jnp.dot(xb, wu_v[:, c * FC:(c + 1) * FC],
                           preferred_element_type=f32)
            anchor(ucol, WTS[1])
            hg = 0.5 * gcol
            hs[c] = ((hg * jnp.tanh(hg) + hg) * ucol).astype(bf16)
        else:
            a = jax.lax.dot_general(ot[0:D, :], wo_v[...], _TN,
                                    preferred_element_type=f32)
            anchor(a, WTS[3])
        if 1 <= c < NF:
            bc = jnp.dot(hs.pop(c - 1), wd_v[(c - 1) * FC:c * FC, :],
                         preferred_element_type=f32)
            anchor(bc, WTS[2])
            b = bc if b is None else b + bc
    gw = gw_ref[...].astype(f32).reshape(1, D)
    z = jnp.sum(xb.astype(f32) * gw, axis=1, keepdims=True)
    gate = 0.5 * jnp.tanh(0.5 * z) + 0.5
    hl = hs.pop(NF - 1)
    for r in range(NO):
        rows = slice(r * RO, (r + 1) * RO)
        br = b[rows] + jnp.dot(hl[rows], wd_v[(NF - 1) * FC:, :],
                               preferred_element_type=f32)
        gr = gate[rows]
        obuf[rows, :] = (br + gr * (a[rows] - br)).astype(obuf.dtype)
        ocopy(step, r).start()

    @pl.when(step == NB - 1)
    def _drain():
        for r in range(NO):
            ocopy(step, r).wait()


@jax.jit
def pallas_gated_mix__grouped_kv_mqa__swiglu_ffn__prompt_kernel(
    A_x: jax.Array,
    A_wq: jax.Array,
    A_wk: jax.Array,
    A_wv: jax.Array,
    A_wo: jax.Array,
    B_x: jax.Array,
    B_w_gate: jax.Array,
    B_w_up: jax.Array,
    B_w_down: jax.Array,
    gate_w: jax.Array,
):
    del B_x
    bf16, f32, u32 = jnp.bfloat16, jnp.float32, jnp.uint32
    any_spec = pl.BlockSpec(memory_space=pl.ANY)
    out = pl.pallas_call(
        _kernel,
        grid=(NB,),
        in_specs=[any_spec] * 8 + [pl.BlockSpec((D,), lambda i: (0,))],
        out_specs=any_spec,
        out_shape=jax.ShapeDtypeStruct((S, D), A_x.dtype),
        scratch_shapes=[
            pltpu.VMEM((S + 16, D), bf16),
            pltpu.VMEM((D, D), bf16),
            pltpu.VMEM((DH, D), bf16),
            pltpu.VMEM((DH, D), bf16),
            pltpu.VMEM((D, D), bf16),
            pltpu.VMEM((D, F), bf16),
            pltpu.VMEM((D, F), bf16),
            pltpu.VMEM((F, D), bf16),
            pltpu.VMEM((S // 2, DH), u32),
            pltpu.VMEM((DH // 2, S), u32),
            pltpu.VMEM(((NC + NBIG) * R, DH * 128), f32),
            pltpu.VMEM((NB, H, DH, TB), bf16),
            pltpu.VMEM((NB, H, DH, TB), f32),
            pltpu.VMEM((D + DH, TB), bf16),
            pltpu.VMEM((LAG, TK, TB), bf16),
            pltpu.VMEM((DH, TB), f32),
            pltpu.VMEM((8, TB), f32),
            pltpu.VMEM((H, NBIG * R, TB), f32),
            pltpu.VMEM((TB, D), bf16),
            pltpu.SMEM((1,), jnp.int32),
            pltpu.SemaphoreType.DMA((17 + NO,)),
        ],
        compiler_params=pltpu.CompilerParams(
            dimension_semantics=("arbitrary",),
            vmem_limit_bytes=100 * 1024 * 1024,
        ),
    )(A_x.reshape(S, D), A_wq, A_wk.T, A_wv.T, A_wo,
      B_w_gate, B_w_up, B_w_down, gate_w)
    return out.reshape(A_x.shape)
```

```python
import math

import jax
import jax.numpy as jnp
import jax.experimental.pallas as pl
import jax.experimental.pallas.tpu as pltpu

S = 2048
D = 512
H = 32
DH = 16
F = 1792

TB = 512
NB = S // TB
NL = TB // 128
TK = 128
NC = S // TK
G = 8
LAG = 2
FC = 256
NF = F // FC
NO = 4
RO = TB // NO

R = 16
BIG = (1, 3, 5, 8, 10, 12, 14)
NBIG = len(BIG)
TSPL = (2, 2, 2, 1)
POS = (4, 7, 10, 13)
POSB = (4, 6, 9, 11)
WTS = (3, 3, 3, 5)
NQS = (8, 12, 12)

SPLIT = 32

QSCALE = (DH ** -0.5) * math.log2(math.e)
SAFE_S = 48.0
SAFE_V = 2.0 ** 60

_NT = (((1,), (1,)), ((), ()))
_TN = (((0,), (0,)), ((), ()))


def rev16(a):
    return jnp.concatenate(
        [a[r:r + 16] for r in range(a.shape[0] - 16, -1, -16)], axis=0)


def _kernel(x_hbm, wq_hbm, wkt_hbm, wvt_hbm, wo_hbm, wg_hbm, wu_hbm, wd_hbm,
            gw_ref, o_hbm,
            x_v, wq_v, wkt_v, wvt_v, wo_v, wg_v, wu_v, wd_v,
            kn, vt, kb, qt16, qf32, ot,
            p_car, o_car, l_car, s_pre, obuf, safe_ref, sems):
    step = pl.program_id(0)
    f32, bf16, u32 = jnp.float32, jnp.bfloat16, jnp.uint32

    srcs = (wkt_hbm, wvt_hbm, wo_hbm, wg_hbm, wu_hbm, wd_hbm)
    dsts = (wkt_v, wvt_v, wo_v, wg_v, wu_v, wd_v)

    def copy(i):
        return pltpu.make_async_copy(srcs[i], dsts[i], sems.at[i])

    def xcopy(b):
        return pltpu.make_async_copy(x_hbm.at[pl.ds(b * TB, TB), :],
                                     x_v.at[pl.ds(b * TB, TB), :],
                                     sems.at[5 + b])

    def stage(k):
        ks = pl.ds(k * 128, 128)
        return (pltpu.make_async_copy(x_hbm.at[pl.ds(0, TB), ks],
                                      x_v.at[pl.ds(0, TB), ks],
                                      sems.at[9 + 2 * k]),
                pltpu.make_async_copy(wq_hbm.at[ks, :], wq_v.at[ks, :],
                                      sems.at[10 + 2 * k]))

    def ocopy(blk, r):
        return pltpu.make_async_copy(
            obuf.at[pl.ds(r * RO, RO), :],
            o_hbm.at[pl.ds(pl.multiple_of(blk * TB + r * RO, RO), RO), :],
            sems.at[17 + r])

    never = jax.lax.broadcasted_iota(jnp.int32, (8, 128), 0) < -step

    def vpu_scores(blk, h, slot, n, j, anchors=None):
        rows = slice(slot * R, (slot + n) * R)
        lanes = slice(j * 128, (j + 1) * 128)
        qrow = qf32[blk, h, 0:1, lanes]
        if anchors is not None:
            q8 = jnp.broadcast_to(qrow, (8, 128))
            qrow = jnp.concatenate(
                [w for a in anchors for w in [jnp.where(never, a, q8)] * 2],
                axis=0)

        def dim(d, acc):
            cols = pl.ds(pl.multiple_of(d * 128, 128), 128)
            return acc + kb[rows, cols] * qf32[blk, h, pl.ds(d, 1), lanes]

        return jax.lax.fori_loop(1, DH, dim, kb[rows, 0:128] * qrow,
                                 unroll=True)

    def release(blk, jobs, res):
        nr, ncol = res.shape[0] // 8, res.shape[1] // 128
        total = len(jobs) * NBIG
        for m, (h, j) in enumerate(jobs):
            anchors = []
            for mm in range(m * NBIG, (m + 1) * NBIG):
                r, jn = (mm * nr) // total, mm % ncol
                anchors.append(res[r * 8:(r + 1) * 8, jn * 128:(jn + 1) * 128])
            i0 = 0
            for n in TSPL:
                s_pre[h, i0 * R:(i0 + n) * R, j * 128:(j + 1) * 128] = (
                    vpu_scores(blk, h, NC + i0, n, j, anchors[i0:i0 + n]))
                i0 += n

    @pl.when(step == 0)
    def _prologue():
        for i in range(2):
            copy(i).start()
        later = [stage(k) for k in range(4)] + [
            (xcopy(b),) for b in range(1, NB)]
        for cp in later[0] + later[1]:
            cp.start()
        later = later[2:]
        p_car[...] = jnp.zeros_like(p_car)
        o_car[...] = jnp.zeros_like(o_car)
        l_car[...] = jnp.ones_like(l_car)
        hr = jax.lax.broadcasted_iota(jnp.int32, (H, D), 0)
        hc = jax.lax.broadcasted_iota(jnp.int32, (H, D), 1)
        sel = jnp.where(hr == (hc >> 4), 1.0, 0.0).astype(bf16)
        for i in range(2):
            copy(i).wait()
        wkvt = jnp.concatenate([wkt_v[...], wvt_v[...]], axis=0)
        cpb = TB // TK
        kxe, kn2s, vmaxs, qn2s = [], [], [], []

        def kv_dot(b):
            return jax.lax.dot_general(wkvt, x_v[b * TB:(b + 1) * TB, :], _NT,
                                       preferred_element_type=f32)

        def kv_block(b, kvt):
            vt[:, b * TB:(b + 1) * TB] = pltpu.bitcast(
                kvt[DH:, :].astype(bf16), u32)
            vmaxs.append(jnp.max(jnp.abs(kvt[DH:, :]), axis=0, keepdims=True))
            kt = kvt[:DH, :].astype(bf16).astype(f32)
            kn2s.append(jnp.sum(kt * kt, axis=0, keepdims=True))
            kxf = kt.T
            kx = kxf.astype(bf16)
            kxr = jnp.concatenate(
                [rev16(kx[c * TK:(c + 1) * TK]) for c in range(cpb)], axis=0)
            kn[b * TB // 2:(b + 1) * TB // 2, :] = pltpu.bitcast(kxr, u32)
            for c in range(cpb):
                cg = b * cpb + c
                r2 = c * TK + R
                vpu_rows = [(cg, c * TK)]
                if cg in BIG:
                    kxe.append(kx[r2:r2 + R, :])
                    vpu_rows.append((NC + BIG.index(cg), r2))
                for slot, r0 in vpu_rows:
                    for d in range(DH):
                        kb[slot * R:(slot + 1) * R, d * 128:(d + 1) * 128] = (
                            jnp.broadcast_to(kxf[r0:r0 + R, d:d + 1], (R, 128)))

        nj0 = sum(NQS)
        hv = H - nj0 // NL
        jobs0 = [(h, j) for h in range(hv, H) for j in range(NL)]

        def q_dot(b):
            qt = jax.lax.dot_general(wqt, x_v[b * TB:(b + 1) * TB, :], _NT,
                                     preferred_element_type=f32)
            if b > 1:
                release(0, jobs0[sum(NQS[:b - 2]):sum(NQS[:b - 1])], qt)
            return qt

        def q_block(b, qt):
            qs = (qt * QSCALE).astype(bf16)
            qf = qs.astype(f32)
            qt16[b] = qs.reshape(H, DH, TB)
            qf32[b] = qf.reshape(H, DH, TB)
            return (qf * qf).astype(bf16)

        def q_norm(q2):
            qn2s.append(jnp.dot(sel, q2, preferred_element_type=f32))

        q0 = kvt0 = None
        wqt = []
        for k in range(4):
            for cp in stage(k):
                cp.wait()
            for grp in later[:(1, 2, 1, 1)[k]]:
                for cp in grp:
                    cp.start()
            later = later[(1, 2, 1, 1)[k]:]
            xk = x_v[0:TB, k * 128:(k + 1) * 128]
            wk = wq_v[k * 128:(k + 1) * 128, :]
            qk = jnp.dot(xk, wk, preferred_element_type=f32)
            kk = jax.lax.dot_general(wkvt[:, k * 128:(k + 1) * 128], xk, _NT,
                                     preferred_element_type=f32)
            q0 = qk if k == 0 else q0 + qk
            kvt0 = kk if k == 0 else kvt0 + kk
            wqt.append(wk.T)
            if k == 0:
                x_v[S:S + 16, :] = qk[TB - 16:, :].astype(bf16)
        wqt = jnp.concatenate(wqt, axis=1)
        xcopy(1).wait()
        qt1 = q_dot(1)
        kvt1 = kv_dot(1)
        kv_block(0, kvt0)
        q2s = [q_block(0, q0.T)]
        for b in range(2, NB):
            xcopy(b).wait()
        for i in range(2, 6):
            copy(i).start()
        kv_block(1, kvt1)
        for b in range(2, NB):
            kv_block(b, kv_dot(b))
        qt2 = q_dot(2)
        q2s.append(q_block(1, qt1))
        q_norm(q2s[0])
        qt3 = q_dot(3)
        q2s.append(q_block(2, qt2))
        q_norm(q2s[1])
        ke = jnp.concatenate(kxe, axis=0)
        rest = jobs0[sum(NQS[:2]):]
        h0 = 8
        for h in range(hv):
            se = jnp.dot(ke, qt16[0, h], preferred_element_type=f32)
            s_pre[h] = se
            if h >= h0:
                release(0, rest[(h - h0) * len(rest) // (hv - 2 - h0):
                                (h - h0 + 1) * len(rest) // (hv - 2 - h0)], se)
            if h == 3:
                q_norm(q2s[2])
            if h == 4:
                q2s.append(q_block(3, qt3))
            if h == 10:
                q_norm(q2s[3])

        def tmax(xs):
            while len(xs) > 1:
                xs = [jnp.maximum(xs[i], xs[i + 1])
                      for i in range(0, len(xs), 2)]
            return jnp.max(xs[0])

        s2 = tmax(qn2s) * tmax(kn2s) * (1.0 + 2.0 ** -5)
        safe = jnp.logical_and(s2 <= SAFE_S * SAFE_S, tmax(vmaxs) <= SAFE_V)
        safe_ref[0] = safe.astype(jnp.int32)

    def k_rows(r0, n):
        return pltpu.bitcast(kn[pl.ds(r0 // 2, n // 2), :], bf16)

    def pv_dot(c, p):
        return jnp.dot(pltpu.bitcast(vt[:, c * TK:(c + 1) * TK], bf16), p,
                       preferred_element_type=f32)

    def finish(o, l, hrow):
        l = l.sum(axis=0, keepdims=True)
        r = pl.reciprocal(l, approx=True)
        o = o * (r * (2.0 - l * r))
        ot[pl.ds(hrow, DH), :] = o.astype(bf16)

    def attn_body(it, carry):
        ps, lsum = {}, {}
        osum = {-1: o_car[...]}
        T = G * NC

        for t in range(T):
            g, c = divmod(t, NC)
            h = it * G + g
            big = c in BIG
            nm = TK - (2 * R if big else R)

            def qk(r0, r1):
                return jnp.dot(k_rows(c * TK + r0, r1 - r0), qt16[step, h],
                               preferred_element_type=f32)

            sa = qk(0, SPLIT)
            g2, c2 = divmod(t - LAG, NC)
            pv = pv_dot(c2, ps.pop(t - LAG) if t >= LAG else p_car[t])
            osum[g2] = pv + osum[g2] if c2 else pv
            if c2 == NC - 1:
                if g2 >= 0:
                    l = lsum.pop(g2)
                    hrow = (it * G + g2) * DH
                else:
                    l = l_car[...]
                    hrow = jnp.where(it == 0, H * DH, (it * G - 1) * DH)
                finish(osum.pop(g2), l, pl.multiple_of(hrow, DH))
            pm = jnp.exp2(jnp.concatenate([sa, qk(SPLIT, nm)], axis=0))
            if c == 0:
                sv = jnp.concatenate(
                    [vpu_scores(step, h, 0, NC, j) for j in range(NL)], axis=1)
            off = [jnp.exp2(sv[c * R:(c + 1) * R])]
            if big:
                i = BIG.index(c)
                pe = jnp.exp2(s_pre[h, i * R:(i + 1) * R, :])
                off.append(pe)
            pos = POSB if big else POS
            acc = lsum.get(g)
            for n in range(nm // 8):
                if big and n == 1:
                    acc = acc + pe[0:8] + pe[8:16]
                if n in pos:
                    j = pos.index(n)
                    w = off[0][:, j * 128:(j + 1) * 128]
                    parts = [acc[:, j * 128:(j + 1) * 128] + w[0:8] + w[8:16]]
                    if j:
                        parts.insert(0, acc[:, :j * 128])
                    if j + 1 < NL:
                        parts.append(acc[:, (j + 1) * 128:])
                    acc = jnp.concatenate(parts, axis=1)
                v = pm[n * 8:(n + 1) * 8, :]
                acc = v if acc is None else acc + v
            lsum[g] = acc
            ps[t] = jnp.concatenate(off + [rev16(pm)], axis=0).astype(bf16)
        for n in range(LAG):
            p_car[n] = ps.pop(T - LAG + n)
        o_car[...] = osum.pop(G - 1)
        l_car[...] = lsum.pop(G - 1)
        return carry

    @pl.when(safe_ref[0] == 1)
    def _fast():
        jax.lax.fori_loop(0, H // G, attn_body, 0)

    @pl.when(safe_ref[0] != 1)
    def _slow():
        def head(h, carry):
            q = qt16[step, h]

            def scores(c):
                return jnp.dot(k_rows(pl.multiple_of(c * TK, TK), TK), q,
                               preferred_element_type=f32)

            def pass1(c, m):
                return jnp.maximum(
                    m, jnp.max(scores(c), axis=0, keepdims=True))

            m = jax.lax.fori_loop(0, NC, pass1,
                                  jnp.full((1, TB), -jnp.inf, f32))

            def pass2(c, ol):
                p = rev16(jnp.exp2(scores(c) - m))
                vc = vt[:, pl.ds(pl.multiple_of(c * TK, TK), TK)]
                pv = jnp.dot(pltpu.bitcast(vc, bf16), p.astype(bf16),
                             preferred_element_type=f32)
                return (ol[0] + pv,
                        ol[1] + p.reshape(TK // 8, 8, TB).sum(axis=0))

            o, l = jax.lax.fori_loop(
                0, NC, pass2,
                (jnp.zeros((DH, TB), f32), jnp.zeros((8, TB), f32)))
            finish(o, l, pl.multiple_of(h * DH, DH))
            o_car[...] = o
            l_car[...] = l
            return carry

        jax.lax.fori_loop(0, H, head, 0)

    @pl.when(step == 0)
    def _wait_weights():
        for i in range(2, 6):
            copy(i).wait()

    @pl.when(step > 0)
    def _wait_out():
        for r in range(NO):
            ocopy(step - 1, r).wait()

    xb = x_v[pl.ds(pl.multiple_of(step * TB, TB), TB), :]
    nxt = jnp.minimum(step + 1, NB - 1)
    jobs = [(h, j) for h in range(H) for j in range(NL)]
    total_w = NF * (WTS[0] + WTS[1] + WTS[2]) - WTS[2] + WTS[3]
    state = {'done': 0, 'w': 0}

    def anchor(res, w):
        state['w'] += w
        upto = len(jobs) * state['w'] // total_w
        release(nxt, jobs[state['done']:upto], res)
        state['done'] = upto

    b = None
    hs = {}
    for c in range(NF + 1):
        if c < NF:
            gcol = jnp.dot(xb, wg_v[:, c * FC:(c + 1) * FC],
                           preferred_element_type=f32)
            anchor(gcol, WTS[0])
            if c == 0:
                o = o_car[...]
                for n in range(LAG):
                    o = o + pv_dot(NC - LAG + n, p_car[n])
                finish(o, l_car[...], (H - 1) * DH)
            ucol = jnp.dot(xb, wu_v[:, c * FC:(c + 1) * FC],
                           preferred_element_type=f32)
            anchor(ucol, WTS[1])
            hg = 0.5 * gcol
            hs[c] = ((hg * jnp.tanh(hg) + hg) * ucol).astype(bf16)
        else:
            a = jax.lax.dot_general(ot[0:D, :], wo_v[...], _TN,
                                    preferred_element_type=f32)
            anchor(a, WTS[3])
        if 1 <= c < NF:
            bc = jnp.dot(hs.pop(c - 1), wd_v[(c - 1) * FC:c * FC, :],
                         preferred_element_type=f32)
            anchor(bc, WTS[2])
            b = bc if b is None else b + bc
    gw = gw_ref[...].astype(f32).reshape(1, D)
    z = jnp.sum(xb.astype(f32) * gw, axis=1, keepdims=True)
    gate = 0.5 * jnp.tanh(0.5 * z) + 0.5
    hl = hs.pop(NF - 1)
    for r in range(NO):
        rows = slice(r * RO, (r + 1) * RO)
        br = b[rows] + jnp.dot(hl[rows], wd_v[(NF - 1) * FC:, :],
                               preferred_element_type=f32)
        gr = gate[rows]
        obuf[rows, :] = (br + gr * (a[rows] - br)).astype(obuf.dtype)
        ocopy(step, r).start()

    @pl.when(step == NB - 1)
    def _drain():
        for r in range(NO):
            ocopy(step, r).wait()


@jax.jit
def pallas_gated_mix__grouped_kv_mqa__swiglu_ffn__prompt_kernel(
    A_x: jax.Array,
    A_wq: jax.Array,
    A_wk: jax.Array,
    A_wv: jax.Array,
    A_wo: jax.Array,
    B_x: jax.Array,
    B_w_gate: jax.Array,
    B_w_up: jax.Array,
    B_w_down: jax.Array,
    gate_w: jax.Array,
):
    del B_x
    bf16, f32, u32 = jnp.bfloat16, jnp.float32, jnp.uint32
    any_spec = pl.BlockSpec(memory_space=pl.ANY)
    out = pl.pallas_call(
        _kernel,
        grid=(NB,),
        in_specs=[any_spec] * 8 + [pl.BlockSpec((D,), lambda i: (0,))],
        out_specs=any_spec,
        out_shape=jax.ShapeDtypeStruct((S, D), A_x.dtype),
        scratch_shapes=[
            pltpu.VMEM((S + 16, D), bf16),
            pltpu.VMEM((D, D), bf16),
            pltpu.VMEM((DH, D), bf16),
            pltpu.VMEM((DH, D), bf16),
            pltpu.VMEM((D, D), bf16),
            pltpu.VMEM((D, F), bf16),
            pltpu.VMEM((D, F), bf16),
            pltpu.VMEM((F, D), bf16),
            pltpu.VMEM((S // 2, DH), u32),
            pltpu.VMEM((DH // 2, S), u32),
            pltpu.VMEM(((NC + NBIG) * R, DH * 128), f32),
            pltpu.VMEM((NB, H, DH, TB), bf16),
            pltpu.VMEM((NB, H, DH, TB), f32),
            pltpu.VMEM((D + DH, TB), bf16),
            pltpu.VMEM((LAG, TK, TB), bf16),
            pltpu.VMEM((DH, TB), f32),
            pltpu.VMEM((8, TB), f32),
            pltpu.VMEM((H, NBIG * R, TB), f32),
            pltpu.VMEM((TB, D), bf16),
            pltpu.SMEM((1,), jnp.int32),
            pltpu.SemaphoreType.DMA((17 + NO,)),
        ],
        compiler_params=pltpu.CompilerParams(
            dimension_semantics=("arbitrary",),
            vmem_limit_bytes=100 * 1024 * 1024,
        ),
    )(A_x.reshape(S, D), A_wq, A_wk.T, A_wv.T, A_wo,
      B_w_gate, B_w_up, B_w_down, gate_w)
    return out.reshape(A_x.shape)
```

```python
import math

import jax
import jax.numpy as jnp
import jax.experimental.pallas as pl
import jax.experimental.pallas.tpu as pltpu

S = 2048
D = 512
H = 32
DH = 16
F = 1792

TB = 512
NB = S // TB
NL = TB // 128
TK = 128
NC = S // TK
G = 8
LAG = 2
FC = 256
NF = F // FC
NO = 4
RO = TB // NO

R = 16
BIG = (1, 3, 5, 8, 10, 12, 14)
NBIG = len(BIG)
TSPL = (2, 2, 2, 1)
POS = (4, 7, 10, 13)
POSB = (4, 6, 9, 11)
WTS = (3, 3, 3, 5)
NQS = (2, 12, 14)

SPLIT = 32

QSCALE = (DH ** -0.5) * math.log2(math.e)
SAFE_S = 48.0
SAFE_V = 2.0 ** 60

_NT = (((1,), (1,)), ((), ()))
_TN = (((0,), (0,)), ((), ()))


def rev16(a):
    return jnp.concatenate(
        [a[r:r + 16] for r in range(a.shape[0] - 16, -1, -16)], axis=0)


def _kernel(x_hbm, wq_hbm, wkt_hbm, wvt_hbm, wo_hbm, wg_hbm, wu_hbm, wd_hbm,
            gw_ref, o_hbm,
            x_v, wq_v, wkt_v, wvt_v, wo_v, wg_v, wu_v, wd_v,
            kn, vt, kb, qt16, qf32, ot,
            p_car, o_car, l_car, s_pre, obuf, safe_ref, sems):
    step = pl.program_id(0)
    f32, bf16, u32 = jnp.float32, jnp.bfloat16, jnp.uint32

    srcs = (wkt_hbm, wvt_hbm, wo_hbm, wg_hbm, wu_hbm, wd_hbm)
    dsts = (wkt_v, wvt_v, wo_v, wg_v, wu_v, wd_v)

    def copy(i):
        return pltpu.make_async_copy(srcs[i], dsts[i], sems.at[i])

    def xcopy(b):
        return pltpu.make_async_copy(x_hbm.at[pl.ds(b * TB, TB), :],
                                     x_v.at[pl.ds(b * TB, TB), :],
                                     sems.at[5 + b])

    def stage(k):
        ks = pl.ds(k * 128, 128)
        return (pltpu.make_async_copy(x_hbm.at[pl.ds(0, TB), ks],
                                      x_v.at[pl.ds(0, TB), ks],
                                      sems.at[9 + 2 * k]),
                pltpu.make_async_copy(wq_hbm.at[ks, :], wq_v.at[ks, :],
                                      sems.at[10 + 2 * k]))

    def ocopy(blk, r):
        return pltpu.make_async_copy(
            obuf.at[pl.ds(r * RO, RO), :],
            o_hbm.at[pl.ds(pl.multiple_of(blk * TB + r * RO, RO), RO), :],
            sems.at[17 + r])

    never = jax.lax.broadcasted_iota(jnp.int32, (8, 128), 0) < -step

    def vpu_scores(blk, h, slot, n, j, anchors=None):
        rows = slice(slot * R, (slot + n) * R)
        lanes = slice(j * 128, (j + 1) * 128)
        qrow = qf32[blk, h, 0:1, lanes]
        if anchors is not None:
            q8 = jnp.broadcast_to(qrow, (8, 128))
            qrow = jnp.concatenate(
                [w for a in anchors for w in [jnp.where(never, a, q8)] * 2],
                axis=0)

        def dim(d, acc):
            cols = pl.ds(pl.multiple_of(d * 128, 128), 128)
            return acc + kb[rows, cols] * qf32[blk, h, pl.ds(d, 1), lanes]

        return jax.lax.fori_loop(1, DH, dim, kb[rows, 0:128] * qrow,
                                 unroll=True)

    def release(blk, jobs, res):
        nr, ncol = res.shape[0] // 8, res.shape[1] // 128
        total = len(jobs) * NBIG
        for m, (h, j) in enumerate(jobs):
            anchors = []
            for mm in range(m * NBIG, (m + 1) * NBIG):
                r, jn = (mm * nr) // total, mm % ncol
                anchors.append(res[r * 8:(r + 1) * 8, jn * 128:(jn + 1) * 128])
            i0 = 0
            for n in TSPL:
                s_pre[h, i0 * R:(i0 + n) * R, j * 128:(j + 1) * 128] = (
                    vpu_scores(blk, h, NC + i0, n, j, anchors[i0:i0 + n]))
                i0 += n

    @pl.when(step == 0)
    def _prologue():
        for i in range(2):
            copy(i).start()
        later = [stage(k) for k in range(4)] + [
            (xcopy(b),) for b in range(1, NB)]
        for cp in later[0] + later[1]:
            cp.start()
        later = later[2:]
        p_car[...] = jnp.zeros_like(p_car)
        o_car[...] = jnp.zeros_like(o_car)
        l_car[...] = jnp.ones_like(l_car)
        for i in range(2):
            copy(i).wait()
        wkvt = jnp.concatenate([wkt_v[...], wvt_v[...]], axis=0)
        cpb = TB // TK
        kxe, kn2s, vmaxs, qn2s = [], [], [], []

        def kv_dot(b):
            return jax.lax.dot_general(wkvt, x_v[b * TB:(b + 1) * TB, :], _NT,
                                       preferred_element_type=f32)

        def kv_block(b, kvt):
            vt[:, b * TB:(b + 1) * TB] = pltpu.bitcast(
                kvt[DH:, :].astype(bf16), u32)
            vmaxs.append(jnp.max(jnp.abs(kvt[DH:, :]), axis=0, keepdims=True))
            kt = kvt[:DH, :].astype(bf16).astype(f32)
            kn2s.append(jnp.sum(kt * kt, axis=0, keepdims=True))
            kxf = kt.T
            kx = kxf.astype(bf16)
            kxr = jnp.concatenate(
                [rev16(kx[c * TK:(c + 1) * TK]) for c in range(cpb)], axis=0)
            kn[b * TB // 2:(b + 1) * TB // 2, :] = pltpu.bitcast(kxr, u32)
            for c in range(cpb):
                cg = b * cpb + c
                r2 = c * TK + R
                vpu_rows = [(cg, c * TK)]
                if cg in BIG:
                    kxe.append(kx[r2:r2 + R, :])
                    vpu_rows.append((NC + BIG.index(cg), r2))
                for slot, r0 in vpu_rows:
                    for d in range(DH):
                        kb[slot * R:(slot + 1) * R, d * 128:(d + 1) * 128] = (
                            jnp.broadcast_to(kxf[r0:r0 + R, d:d + 1], (R, 128)))

        nj0 = sum(NQS)
        hv = H - nj0 // NL
        jobs0 = [(h, j) for h in range(hv, H) for j in range(NL)]

        def q_dot(b):
            qt = jax.lax.dot_general(wqt, x_v[b * TB:(b + 1) * TB, :], _NT,
                                     preferred_element_type=f32)
            if b > 1:
                release(0, jobs0[sum(NQS[:b - 2]):sum(NQS[:b - 1])], qt)
            return qt

        def q_block(b, qt):
            qs = (qt * QSCALE).astype(bf16)
            qf = qs.astype(f32)
            qt16[b] = qs.reshape(H, DH, TB)
            qf32[b] = qf.reshape(H, DH, TB)
            q2 = (qf * qf).reshape(H, 2, 8, TB)
            qn2s.append(8.0 * jnp.max(q2[:, 0] + q2[:, 1], axis=0))

        q0 = kvt0 = None
        wqt = []
        for k in range(4):
            for cp in stage(k):
                cp.wait()
            for grp in later[:(1, 2, 1, 1)[k]]:
                for cp in grp:
                    cp.start()
            later = later[(1, 2, 1, 1)[k]:]
            xk = x_v[0:TB, k * 128:(k + 1) * 128]
            wk = wq_v[k * 128:(k + 1) * 128, :]
            qk = jnp.dot(xk, wk, preferred_element_type=f32)
            kk = jax.lax.dot_general(wkvt[:, k * 128:(k + 1) * 128], xk, _NT,
                                     preferred_element_type=f32)
            q0 = qk if k == 0 else q0 + qk
            kvt0 = kk if k == 0 else kvt0 + kk
            wqt.append(wk.T)
            if k == 0:
                x_v[S:S + 16, :] = qk[TB - 16:, :].astype(bf16)
        wqt = jnp.concatenate(wqt, axis=1)
        xcopy(1).wait()
        qt1 = q_dot(1)
        kvt1 = kv_dot(1)
        kv_block(0, kvt0)
        q_block(0, q0.T)
        for b in range(2, NB):
            xcopy(b).wait()
        for i in range(2, 6):
            copy(i).start()
        kv_block(1, kvt1)
        for b in range(2, NB):
            kv_block(b, kv_dot(b))
        qt2 = q_dot(2)
        q_block(1, qt1)
        qt3 = q_dot(3)
        q_block(2, qt2)
        ke = jnp.concatenate(kxe, axis=0)
        rest = jobs0[sum(NQS[:2]):]
        h0 = 4
        for h in range(hv):
            se = jnp.dot(ke, qt16[0, h], preferred_element_type=f32)
            s_pre[h] = se
            if h >= h0:
                release(0, rest[(h - h0) * len(rest) // (hv - 2 - h0):
                                (h - h0 + 1) * len(rest) // (hv - 2 - h0)], se)
            if h == 2:
                q_block(3, qt3)

        def tmax(xs):
            while len(xs) > 1:
                xs = [jnp.maximum(xs[i], xs[i + 1])
                      for i in range(0, len(xs), 2)]
            return jnp.max(xs[0])

        s2 = tmax(qn2s) * tmax(kn2s) * (1.0 + 2.0 ** -5)
        safe = jnp.logical_and(s2 <= SAFE_S * SAFE_S, tmax(vmaxs) <= SAFE_V)
        safe_ref[0] = safe.astype(jnp.int32)

    def k_rows(r0, n):
        return pltpu.bitcast(kn[pl.ds(r0 // 2, n // 2), :], bf16)

    def pv_dot(c, p):
        return jnp.dot(pltpu.bitcast(vt[:, c * TK:(c + 1) * TK], bf16), p,
                       preferred_element_type=f32)

    def finish(o, l, hrow):
        l = l.sum(axis=0, keepdims=True)
        r = pl.reciprocal(l, approx=True)
        o = o * (r * (2.0 - l * r))
        ot[pl.ds(hrow, DH), :] = o.astype(bf16)

    def attn_body(it, carry):
        ps, lsum = {}, {}
        osum = {-1: o_car[...]}
        T = G * NC

        for t in range(T):
            g, c = divmod(t, NC)
            h = it * G + g
            big = c in BIG
            nm = TK - (2 * R if big else R)

            def qk(r0, r1):
                return jnp.dot(k_rows(c * TK + r0, r1 - r0), qt16[step, h],
                               preferred_element_type=f32)

            sa = qk(0, SPLIT)
            g2, c2 = divmod(t - LAG, NC)
            pv = pv_dot(c2, ps.pop(t - LAG) if t >= LAG else p_car[t])
            osum[g2] = pv + osum[g2] if c2 else pv
            if c2 == NC - 1:
                if g2 >= 0:
                    l = lsum.pop(g2)
                    hrow = (it * G + g2) * DH
                else:
                    l = l_car[...]
                    hrow = jnp.where(it == 0, H * DH, (it * G - 1) * DH)
                finish(osum.pop(g2), l, pl.multiple_of(hrow, DH))
            pm = jnp.exp2(jnp.concatenate([sa, qk(SPLIT, nm)], axis=0))
            if c == 0:
                sv = jnp.concatenate(
                    [vpu_scores(step, h, 0, NC, j) for j in range(NL)], axis=1)
            off = [jnp.exp2(sv[c * R:(c + 1) * R])]
            if big:
                i = BIG.index(c)
                pe = jnp.exp2(s_pre[h, i * R:(i + 1) * R, :])
                off.append(pe)
            pos = POSB if big else POS
            acc = lsum.get(g)
            for n in range(nm // 8):
                if big and n == 1:
                    acc = acc + pe[0:8] + pe[8:16]
                if n in pos:
                    j = pos.index(n)
                    w = off[0][:, j * 128:(j + 1) * 128]
                    parts = [acc[:, j * 128:(j + 1) * 128] + w[0:8] + w[8:16]]
                    if j:
                        parts.insert(0, acc[:, :j * 128])
                    if j + 1 < NL:
                        parts.append(acc[:, (j + 1) * 128:])
                    acc = jnp.concatenate(parts, axis=1)
                v = pm[n * 8:(n + 1) * 8, :]
                acc = v if acc is None else acc + v
            lsum[g] = acc
            ps[t] = jnp.concatenate(off + [rev16(pm)], axis=0).astype(bf16)
        for n in range(LAG):
            p_car[n] = ps.pop(T - LAG + n)
        o_car[...] = osum.pop(G - 1)
        l_car[...] = lsum.pop(G - 1)
        return carry

    def _fast():
        jax.lax.fori_loop(0, H // G, attn_body, 0)

    def _slow():
        def head(h, carry):
            q = qt16[step, h]

            def scores(c):
                return jnp.dot(k_rows(pl.multiple_of(c * TK, TK), TK), q,
                               preferred_element_type=f32)

            def pass1(c, m):
                return jnp.maximum(
                    m, jnp.max(scores(c), axis=0, keepdims=True))

            m = jax.lax.fori_loop(0, NC, pass1,
                                  jnp.full((1, TB), -jnp.inf, f32))

            def pass2(c, ol):
                p = rev16(jnp.exp2(scores(c) - m))
                vc = vt[:, pl.ds(pl.multiple_of(c * TK, TK), TK)]
                pv = jnp.dot(pltpu.bitcast(vc, bf16), p.astype(bf16),
                             preferred_element_type=f32)
                return (ol[0] + pv,
                        ol[1] + p.reshape(TK // 8, 8, TB).sum(axis=0))

            o, l = jax.lax.fori_loop(
                0, NC, pass2,
                (jnp.zeros((DH, TB), f32), jnp.zeros((8, TB), f32)))
            finish(o, l, pl.multiple_of(h * DH, DH))
            o_car[...] = o
            l_car[...] = l
            return carry

        jax.lax.fori_loop(0, H, head, 0)

    jax.lax.cond(safe_ref[0] == 1, _fast, _slow)

    @pl.when(step == 0)
    def _wait_weights():
        for i in range(2, 6):
            copy(i).wait()

    @pl.when(step > 0)
    def _wait_out():
        for r in range(NO):
            ocopy(step - 1, r).wait()

    xb = x_v[pl.ds(pl.multiple_of(step * TB, TB), TB), :]
    nxt = jnp.minimum(step + 1, NB - 1)
    jobs = [(h, j) for h in range(H) for j in range(NL)]
    total_w = NF * (WTS[0] + WTS[1] + WTS[2]) - WTS[2] + WTS[3]
    state = {'done': 0, 'w': 0}

    def anchor(res, w):
        state['w'] += w
        upto = len(jobs) * state['w'] // total_w
        release(nxt, jobs[state['done']:upto], res)
        state['done'] = upto

    b = None
    hs = {}
    for c in range(NF + 1):
        if c < NF:
            gcol = jnp.dot(xb, wg_v[:, c * FC:(c + 1) * FC],
                           preferred_element_type=f32)
            anchor(gcol, WTS[0])
            if c == 0:
                o = o_car[...]
                for n in range(LAG):
                    o = o + pv_dot(NC - LAG + n, p_car[n])
                finish(o, l_car[...], (H - 1) * DH)
            ucol = jnp.dot(xb, wu_v[:, c * FC:(c + 1) * FC],
                           preferred_element_type=f32)
            anchor(ucol, WTS[1])
            hg = 0.5 * gcol
            hs[c] = ((hg * jnp.tanh(hg) + hg) * ucol).astype(bf16)
        else:
            a = jax.lax.dot_general(ot[0:D, :], wo_v[...], _TN,
                                    preferred_element_type=f32)
            anchor(a, WTS[3])
        if 1 <= c < NF:
            bc = jnp.dot(hs.pop(c - 1), wd_v[(c - 1) * FC:c * FC, :],
                         preferred_element_type=f32)
            anchor(bc, WTS[2])
            b = bc if b is None else b + bc
    gw = gw_ref[...].astype(f32).reshape(1, D)
    z = jnp.sum(xb.astype(f32) * gw, axis=1, keepdims=True)
    gate = 0.5 * jnp.tanh(0.5 * z) + 0.5
    hl = hs.pop(NF - 1)
    for r in range(NO):
        rows = slice(r * RO, (r + 1) * RO)
        br = b[rows] + jnp.dot(hl[rows], wd_v[(NF - 1) * FC:, :],
                               preferred_element_type=f32)
        gr = gate[rows]
        obuf[rows, :] = (br + gr * (a[rows] - br)).astype(obuf.dtype)
        ocopy(step, r).start()

    @pl.when(step == NB - 1)
    def _drain():
        for r in range(NO):
            ocopy(step, r).wait()


@jax.jit
def pallas_gated_mix__grouped_kv_mqa__swiglu_ffn__prompt_kernel(
    A_x: jax.Array,
    A_wq: jax.Array,
    A_wk: jax.Array,
    A_wv: jax.Array,
    A_wo: jax.Array,
    B_x: jax.Array,
    B_w_gate: jax.Array,
    B_w_up: jax.Array,
    B_w_down: jax.Array,
    gate_w: jax.Array,
):
    del B_x
    bf16, f32, u32 = jnp.bfloat16, jnp.float32, jnp.uint32
    any_spec = pl.BlockSpec(memory_space=pl.ANY)
    out = pl.pallas_call(
        _kernel,
        grid=(NB,),
        in_specs=[any_spec] * 8 + [pl.BlockSpec((D,), lambda i: (0,))],
        out_specs=any_spec,
        out_shape=jax.ShapeDtypeStruct((S, D), A_x.dtype),
        scratch_shapes=[
            pltpu.VMEM((S + 16, D), bf16),
            pltpu.VMEM((D, D), bf16),
            pltpu.VMEM((DH, D), bf16),
            pltpu.VMEM((DH, D), bf16),
            pltpu.VMEM((D, D), bf16),
            pltpu.VMEM((D, F), bf16),
            pltpu.VMEM((D, F), bf16),
            pltpu.VMEM((F, D), bf16),
            pltpu.VMEM((S // 2, DH), u32),
            pltpu.VMEM((DH // 2, S), u32),
            pltpu.VMEM(((NC + NBIG) * R, DH * 128), f32),
            pltpu.VMEM((NB, H, DH, TB), bf16),
            pltpu.VMEM((NB, H, DH, TB), f32),
            pltpu.VMEM((D + DH, TB), bf16),
            pltpu.VMEM((LAG, TK, TB), bf16),
            pltpu.VMEM((DH, TB), f32),
            pltpu.VMEM((8, TB), f32),
            pltpu.VMEM((H, NBIG * R, TB), f32),
            pltpu.VMEM((TB, D), bf16),
            pltpu.SMEM((1,), jnp.int32),
            pltpu.SemaphoreType.DMA((17 + NO,)),
        ],
        compiler_params=pltpu.CompilerParams(
            dimension_semantics=("arbitrary",),
            vmem_limit_bytes=100 * 1024 * 1024,
        ),
    )(A_x.reshape(S, D), A_wq, A_wk.T, A_wv.T, A_wo,
      B_w_gate, B_w_up, B_w_down, gate_w)
    return out.reshape(A_x.shape)
```
